```python
import jax
import jax.numpy as jnp

def _softmax(x, axis=-1):
    return jax.nn.softmax(x, axis=axis)

def _gelu(x):
    return jax.nn.gelu(x, approximate=True)

def _silu(x):
    return jax.nn.silu(x)

def _sigmoid(x):
    return jax.nn.sigmoid(x)

def _layernorm(x, axis=-1, eps=1e-05):
    m = jnp.mean(x, axis=axis, keepdims=True)
    v = jnp.var(x, axis=axis, keepdims=True)
    return (x - m) / jnp.sqrt(v + eps)

def _scatter_add(tgt, idx, src, axis=0):
    return tgt.at[idx].add(src)

def _segment_sum(src, seg, n):
    return jax.ops.segment_sum(src, seg, n)

class _Rng:

    def __init__(self, key):
        self._k = key

    def _next(self):
        self._k, sub = jax.random.split(self._k)
        return sub

    def normal(self, shape):
        return jax.random.normal(self._next(), shape, dtype=jnp.bfloat16)

    def randint(self, lo, hi, shape):
        return jax.random.randint(self._next(), shape, lo, hi, dtype=jnp.int32)

    def uniform(self, shape, lo=0.0, hi=1.0):
        return jax.random.uniform(self._next(), shape, jnp.bfloat16, lo, hi)

    def permutation(self, n):
        return jax.random.permutation(self._next(), n)
kernel_name = 'adaLN_cond__sliding_block_cached__glu_gated_glu__decode'

def setup_inputs():
    _rng = _Rng(jax.random.key(int.from_bytes(__import__("os").urandom(4), "little")))
    _w = lambda a: (lambda t: t.astype(jnp.bfloat16) if jnp.issubdtype(t.dtype, jnp.floating) else t)(jnp.asarray(a))

    def _A_setup():
        B, Sq, D = (8, 1, 512)
        Hq, Hkv, Sk, Dh = (32, 32, 4096, 128)
        assert Hq % Hkv == 0, (Hq, Hkv)
        return {'x': _w((lambda *s: _rng.normal(s) * 0.05)(B, Sq, D)), 'k_cache': _w((lambda *s: _rng.normal(s) * 0.05)(B, Hkv, Sk, Dh)), 'v_cache': _w((lambda *s: _rng.normal(s) * 0.05)(B, Hkv, Sk, Dh)), 'wq': _w((lambda *s: _rng.normal(s) * 0.05)(D, Hq * Dh) * D ** (-0.5)), 'wo': _w((lambda *s: _rng.normal(s) * 0.05)(Hq * Dh, D) * (Hq * Dh) ** (-0.5))}
    _A_in = _A_setup()

    def _B_setup():
        B, S, D, F = (8, 1, 512, 1376)
        return {'x': _w((lambda *s: _rng.normal(s) * 0.05)(B, S, D)), 'w_gate': _w((lambda *s: _rng.normal(s) * 0.05)(D, F)), 'w_up': _w((lambda *s: _rng.normal(s) * 0.05)(D, F)), 'w_down': _w((lambda *s: _rng.normal(s) * 0.05)(F, D))}
    _B_in = _B_setup()
    return {'A_x': _A_in['x'], 'A_k_cache': _A_in['k_cache'], 'A_v_cache': _A_in['v_cache'], 'A_wq': _A_in['wq'], 'A_wo': _A_in['wo'], 'B_x': _B_in['x'], 'B_w_gate': _B_in['w_gate'], 'B_w_up': _B_in['w_up'], 'B_w_down': _B_in['w_down'], 'c': _w((lambda *s: _rng.normal(s) * 0.05)(8, 512)), 'w_mod': _w((lambda *s: _rng.normal(s) * 0.05)(512, 6 * 512) * 512 ** (-0.5))}

def reference(A_x, A_k_cache, A_v_cache, A_wq, A_wo, B_x, B_w_gate, B_w_up, B_w_down, c, w_mod):

    def _A_ref(x, k_cache, v_cache, wq, wo):
        B, Sq, D = x.shape
        Hq, Dh = (32, 128)
        Hkv, Sk = (k_cache.shape[1], k_cache.shape[2])
        W = min(4096, max(256, Sk // 4))
        rep = Hq // Hkv
        q = (lambda x, *d: x.transpose(*d))((x @ wq).reshape(B, Sq, Hq, Dh), 0, 2, 1, 3)
        k = jnp.repeat(k_cache[:, :, Sk - W:, :], rep, axis=1)
        v = jnp.repeat(v_cache[:, :, Sk - W:, :], rep, axis=1)
        scores = jnp.einsum('bhqd,bhkd->bhqk', q, k) * Dh ** (-0.5)
        p = _softmax(scores, axis=-1)
        o = jnp.einsum('bhqk,bhkd->bhqd', p, v)
        return (lambda x, *d: x.transpose(*d))(o, 0, 2, 1, 3).reshape(B, Sq, Hq * Dh) @ wo

    def _B_ref(x, w_gate, w_up, w_down):
        g = jnp.einsum('bsd,df->bsf', x, w_gate)
        u = jnp.einsum('bsd,df->bsf', x, w_up)
        h = _sigmoid(g) * u
        return jnp.einsum('bsf,fd->bsd', h, w_down)
    x = A_x
    mod = (_silu(c) @ w_mod).reshape(c.shape[0], 6, 1, -1)
    sa, ca, ga, sb, cb, gb = (mod[:, 0].copy(), mod[:, 1].copy(), mod[:, 2].copy(), mod[:, 3].copy(), mod[:, 4].copy(), mod[:, 5].copy())
    h = _layernorm(x, axis=-1) * (1 + ca) + sa
    x = x + ga * _A_ref(h, A_k_cache, A_v_cache, A_wq, A_wo)
    h = _layernorm(x, axis=-1) * (1 + cb) + sb
    x = x + gb * _B_ref(h, B_w_gate, B_w_up, B_w_down)
    return x
```

```python
import functools

import jax
import jax.numpy as jnp
from jax import lax
import jax.experimental.pallas as pl
import jax.experimental.pallas.tpu as pltpu

_F32 = jnp.float32
_BF16 = jnp.bfloat16
_NT = (((1,), (1,)), ((), ()))

_HQ = 32
_DH = 128
_S = 16
_R = 32
_LA = 8
_RING = 16
_EPS = 1e-5


def _layernorm(x):
    m = jnp.mean(x, axis=-1, keepdims=True)
    xc = x - m
    v = jnp.mean(xc * xc, axis=-1, keepdims=True)
    return xc * lax.rsqrt(v + _EPS)


def _sigmoid(x):
    return 1.0 / (1.0 + jnp.exp(-x))


def _kernel(x_hbm, k_hbm, v_hbm, wq_hbm, wo_hbm, wg_hbm, wu_hbm, wd_hbm, c_hbm, wm_hbm,
            out_ref,
            kbuf, vbuf, wm_buf, wq_buf, wo_buf, wg_buf, wu_buf, wd_buf, x_buf, c_buf,
            mod_ref, q_ref, o_ref, s_ref, h_ref, sem, sem2,
            *, B, D, F, Sk, W):
    NG = k_hbm.shape[0]
    NSTEP = W // _R
    GPB = _HQ // _S
    scale = _DH ** -0.5

    def pairs(src_at, dst_at, bank, j, nstreams):
        out = []
        for p in range(nstreams // 8):
            lo = pltpu.make_async_copy(src_at(pl.ds(8 * p, 7)), dst_at(pl.ds(8 * p, 7)),
                                       sem.at[bank, j & (_RING - 1), 2 * p])
            hi = pltpu.make_async_copy(src_at(pl.ds(8 * p + 7, 1)), dst_at(pl.ds(8 * p + 7, 1)),
                                       sem.at[bank, j & (_RING - 1), 2 * p + 1])
            out.append((lo, hi))
        return out

    def kv_step(src, dst, bank, g, j):
        r = pl.multiple_of(j * _R, _R)
        return pairs(lambda s: src.at[g, s, pl.ds(Sk - W + r, _R), :],
                     lambda s: dst.at[s, pl.ds(r, _R), :], bank, j, _S)

    k_step = functools.partial(kv_step, k_hbm, kbuf, 0)
    v_step = functools.partial(kv_step, v_hbm, vbuf, 1)

    def w_step(src, dst, bank, ncb, cw, j):
        out = []
        for p in range(2):
            e = 2 * j + p
            r = pl.multiple_of((e >> (ncb.bit_length() - 1)) * 8, 8)
            if ncb == 1:
                cs = slice(None)
            else:
                cs = pl.ds(pl.multiple_of((e & (ncb - 1)) * cw, 128), cw)
            lo = pltpu.make_async_copy(src.at[pl.ds(0, 7), pl.ds(r, 8), cs], dst.at[pl.ds(0, 7), pl.ds(r, 8), cs],
                                       sem.at[bank, j & (_RING - 1), 2 * p])
            hi = pltpu.make_async_copy(src.at[pl.ds(7, 1), pl.ds(r, 8), cs], dst.at[pl.ds(7, 1), pl.ds(r, 8), cs],
                                       sem.at[bank, j & (_RING - 1), 2 * p + 1])
            out.append((lo, hi))
        return out

    wm_step = functools.partial(w_step, wm_hbm, wm_buf, 0, 4, 6 * D // 4)
    wq_step = functools.partial(w_step, wq_hbm, wq_buf, 1, 8, _HQ * _DH // 8)
    wo_step = functools.partial(w_step, wo_hbm, wo_buf, 0, 1, D)
    N_WM, N_WQ, N_WO = 16, 32, 32

    def start(step):
        for lo, hi in step:
            lo.start(priority=1)
            hi.start(priority=0)

    def advance(wait_step, start_step):
        for p, (lo, hi) in enumerate(wait_step):
            lo.wait()
            if start_step is not None:
                start_step[p][0].start(priority=1)
                start_step[p][1].start(priority=0)
            hi.wait()

    def loop(n, body):
        def f(i, c):
            body(i)
            return c
        lax.fori_loop(0, n, f, 0)

    def phase(cur, n, nxt, compute, nbody, spb):
        def body(i):
            for t in range(spb):
                j = i * spb + t
                advance(cur(j), cur(j + _LA))
                if t == 0:
                    compute(i)
        if nbody:
            loop(nbody, body)
        done = nbody * spb
        if n - _LA > done:
            loop(n - _LA - done, lambda i: advance(cur(done + i), cur(done + i + _LA)))
        loop(_LA, lambda i: advance(cur(n - _LA + i), None if nxt is None else nxt(i)))

    cx = pltpu.make_async_copy(x_hbm, x_buf, sem2.at[0])
    cc = pltpu.make_async_copy(c_hbm, c_buf, sem2.at[1])
    cx.start()
    cc.start()
    loop(_LA, lambda i: start(wm_step(i)))
    phase(wm_step, N_WM, wq_step, None, 0, 0)

    cc.wait()
    cx.wait()
    c = c_buf[...].astype(_F32)
    h_ref[...] = c * _sigmoid(c)

    MB = mod_ref.shape[0]
    MW = mod_ref.shape[2]

    def mod_block(i):
        w = wm_buf[:, :, pl.ds(pl.multiple_of(i * MW, 128), MW)].reshape(D, MW)
        mod_ref[i] = jnp.dot(h_ref[...].astype(_BF16), w, preferred_element_type=_F32)

    phase(wq_step, N_WQ, functools.partial(k_step, 0), mod_block, MB, 2)

    def mod(k):
        per = D // MW
        return jnp.concatenate([mod_ref[k * per + t] for t in range(per)], axis=-1)

    def load_x():
        return x_buf[...].astype(_F32)

    h_ref[...] = _layernorm(load_x()) * (1.0 + mod(1)) + mod(0)

    def q_block(i):
        w = wq_buf[:, :, pl.ds(pl.multiple_of(i * 4 * _DH, 128), 4 * _DH)].reshape(D, 4 * _DH)
        q = jnp.dot(h_ref[...].astype(_BF16), w, preferred_element_type=_F32)
        for t in range(4):
            q_ref[4 * i + t] = q[:, t * _DH:(t + 1) * _DH]

    phase(functools.partial(k_step, 0), NSTEP, functools.partial(v_step, 0), q_block, 8, 3)

    def unit_bh(g, u):
        return g >> (GPB.bit_length() - 1), (g & (GPB - 1)) * _S + u

    def qk(g, i):
        for t in range(2):
            u = 2 * i + t
            b, h = unit_bh(g, u)
            q = q_ref[h, pl.ds(b, 1), :].astype(_BF16)
            s_ref[pl.ds(u, 1), :] = lax.dot_general(q, kbuf[u], _NT, preferred_element_type=_F32)

    def softmax():
        s = s_ref[...] * scale
        m = jnp.max(s, axis=-1, keepdims=True)
        p = jnp.exp(s - m)
        s_ref[...] = p * (1.0 / jnp.sum(p, axis=-1, keepdims=True))

    def pv(g, i):
        for t in range(2):
            u = 2 * i + t
            b, h = unit_bh(g, u)
            p = s_ref[pl.ds(u, 1), :].astype(_BF16)
            o_ref[h, pl.ds(b, 1), :] = jnp.dot(p, vbuf[u], preferred_element_type=_F32)

    def group(g):
        phase(functools.partial(v_step, g), NSTEP, functools.partial(k_step, g + 1),
              functools.partial(qk, g), 8, 3)
        softmax()
        phase(functools.partial(k_step, g + 1), NSTEP, functools.partial(v_step, g + 1),
              functools.partial(pv, g), 8, 3)

    loop(NG - 1, group)
    phase(functools.partial(v_step, NG - 1), NSTEP, wo_step, functools.partial(qk, NG - 1), 8, 3)
    softmax()

    splits = [(0, 512), (512, 512), (1024, 256), (1280, F - 1280)]
    NSP = len(splits)

    def rows_copy(src, dst, t, si):
        r, n = splits[t]
        return pltpu.make_async_copy(src.at[pl.ds(r, n)], dst.at[pl.ds(r, n)], sem2.at[si])
    g_copies = [rows_copy(wg_hbm, wg_buf, t, 2 + t) for t in range(NSP)]
    u_copies = [rows_copy(wu_hbm, wu_buf, t, 2 + NSP + t) for t in range(NSP)]
    d_copies = [rows_copy(wd_hbm, wd_buf, t, 2 + 2 * NSP + t) for t in range(NSP)]

    def wo_body(i):
        for t in range(3):
            j = i * 3 + t
            advance(wo_step(j), wo_step(j + _LA))
            if t == 0:
                pv(NG - 1, i)
    loop(8, wo_body)
    for t in range(NSP):
        g_copies[t].start(priority=1)
        u_copies[t].start(priority=1)
    for t in range(NSP):
        d_copies[t].start(priority=1)
    loop(_LA, lambda i: advance(wo_step(N_WO - _LA + i), None))

    def wo_block(i, acc):
        o = jnp.concatenate([o_ref[4 * i + t] for t in range(4)], axis=-1).astype(_BF16)
        return acc + jnp.dot(o, wo_buf[i], preferred_element_type=_F32)
    attn = lax.fori_loop(0, 8, wo_block, jnp.zeros((B, D), _F32))

    x1 = load_x() + mod(2) * attn
    h2 = (_layernorm(x1) * (1.0 + mod(4)) + mod(3)).astype(_BF16)

    hh = []
    for t, (r, n) in enumerate(splits):
        g_copies[t].wait()
        gate = lax.dot_general(h2, wg_buf[r:r + n, :], _NT, preferred_element_type=_F32)
        u_copies[t].wait()
        up = lax.dot_general(h2, wu_buf[r:r + n, :], _NT, preferred_element_type=_F32)
        hh.append((_sigmoid(gate) * up).astype(_BF16))
    y = jnp.zeros((B, D), _F32)
    for t, (r, n) in enumerate(splits):
        d_copies[t].wait()
        y = y + jnp.dot(hh[t], wd_buf[r:r + n, :], preferred_element_type=_F32)
    out_ref[...] = (x1 + mod(5) * y).astype(out_ref.dtype)


@jax.jit
def pallas_adaLN_cond__sliding_block_cached__glu_gated_glu__decode_kernel(
    A_x: jax.Array,
    A_k_cache: jax.Array,
    A_v_cache: jax.Array,
    A_wq: jax.Array,
    A_wo: jax.Array,
    B_x: jax.Array,
    B_w_gate: jax.Array,
    B_w_up: jax.Array,
    B_w_down: jax.Array,
    c: jax.Array,
    w_mod: jax.Array,
):
    del B_x
    B, Sq, D = A_x.shape
    Hkv, Sk = A_k_cache.shape[1], A_k_cache.shape[2]
    F = B_w_gate.shape[1]
    assert Sq == 1 and Hkv == _HQ and A_k_cache.shape[3] == _DH
    W = min(4096, max(256, Sk // 4))
    NG = B * _HQ // _S

    k = A_k_cache.reshape(NG, _S, Sk, _DH)
    v = A_v_cache.reshape(NG, _S, Sk, _DH)
    wq = A_wq.reshape(8, D // 8, _HQ * _DH)
    wo = A_wo.reshape(8, _HQ * _DH // 8, D)
    wm = w_mod.reshape(8, D // 8, 6 * D)
    x = A_x.reshape(B, D)
    wg = B_w_gate.T
    wu = B_w_up.T

    any_spec = pl.BlockSpec(memory_space=pl.ANY)
    out = pl.pallas_call(
        functools.partial(_kernel, B=B, D=D, F=F, Sk=Sk, W=W),
        out_shape=jax.ShapeDtypeStruct(x.shape, x.dtype),
        in_specs=[any_spec] * 10,
        out_specs=pl.BlockSpec(memory_space=pltpu.VMEM),
        scratch_shapes=[
            pltpu.VMEM((_S, W, _DH), _BF16),
            pltpu.VMEM((_S, W, _DH), _BF16),
            pltpu.VMEM(wm.shape, _BF16),
            pltpu.VMEM(wq.shape, _BF16),
            pltpu.VMEM(wo.shape, _BF16),
            pltpu.VMEM(wg.shape, _BF16),
            pltpu.VMEM(wu.shape, _BF16),
            pltpu.VMEM(B_w_down.shape, _BF16),
            pltpu.VMEM(x.shape, _BF16),
            pltpu.VMEM(c.shape, _BF16),
            pltpu.VMEM((12, B, 6 * D // 12), _F32),
            pltpu.VMEM((_HQ, B, _DH), _F32),
            pltpu.VMEM((_HQ, B, _DH), _F32),
            pltpu.VMEM((_S, W), _F32),
            pltpu.VMEM((B, D), _F32),
            pltpu.SemaphoreType.DMA((2, _RING, 4)),
            pltpu.SemaphoreType.DMA((16,)),
        ],
        compiler_params=pltpu.CompilerParams(
            vmem_limit_bytes=64 * 1024 * 1024,
        ),
    )(x, k, v, wq, wo, wg, wu, B_w_down, c, wm)
    return out.reshape(A_x.shape)
```

```python
import functools

import jax
import jax.numpy as jnp
from jax import lax
import jax.experimental.pallas as pl
import jax.experimental.pallas.tpu as pltpu

_F32 = jnp.float32
_BF16 = jnp.bfloat16
_NT = (((1,), (1,)), ((), ()))

_HQ = 32
_DH = 128
_S = 16
_R = 32
_LA = 8
_RING = 16
_EPS = 1e-5
_FP = 16
_FRING = 32


def _layernorm(x):
    m = jnp.mean(x, axis=-1, keepdims=True)
    xc = x - m
    v = jnp.mean(xc * xc, axis=-1, keepdims=True)
    return xc * lax.rsqrt(v + _EPS)


def _sigmoid(x):
    return 1.0 / (1.0 + jnp.exp(-x))


def _kernel(x_hbm, k_hbm, v_hbm, wq_hbm, wo_hbm, wg_hbm, wu_hbm, wd_hbm, c_hbm, wm_hbm,
            out_ref,
            kbuf, vbuf, wm_buf, wq_buf, wo_buf, wg_buf, wu_buf, wd_buf, x_buf, c_buf,
            mod_ref, q_ref, o_ref, s_ref, h_ref, sem, sem2,
            *, B, D, F, Sk, W):
    NG = k_hbm.shape[0]
    NSTEP = W // _R
    GPB = _HQ // _S
    scale = _DH ** -0.5

    def pairs(src_at, dst_at, bank, j, nstreams):
        out = []
        for p in range(nstreams // 8):
            lo = pltpu.make_async_copy(src_at(pl.ds(8 * p, 7)), dst_at(pl.ds(8 * p, 7)),
                                       sem.at[bank, j & (_RING - 1), 2 * p])
            hi = pltpu.make_async_copy(src_at(pl.ds(8 * p + 7, 1)), dst_at(pl.ds(8 * p + 7, 1)),
                                       sem.at[bank, j & (_RING - 1), 2 * p + 1])
            out.append((lo, hi))
        return out

    def kv_step(src, dst, bank, g, j):
        r = pl.multiple_of(j * _R, _R)
        return pairs(lambda s: src.at[g, s, pl.ds(Sk - W + r, _R), :],
                     lambda s: dst.at[s, pl.ds(r, _R), :], bank, j, _S)

    k_step = functools.partial(kv_step, k_hbm, kbuf, 0)
    v_step = functools.partial(kv_step, v_hbm, vbuf, 1)

    def w_step(src, dst, bank, ncb, cw, j):
        out = []
        for p in range(2):
            e = 2 * j + p
            r = pl.multiple_of((e >> (ncb.bit_length() - 1)) * 8, 8)
            if ncb == 1:
                cs = slice(None)
            else:
                cs = pl.ds(pl.multiple_of((e & (ncb - 1)) * cw, 128), cw)
            lo = pltpu.make_async_copy(src.at[pl.ds(0, 7), pl.ds(r, 8), cs], dst.at[pl.ds(0, 7), pl.ds(r, 8), cs],
                                       sem.at[bank, j & (_RING - 1), 2 * p])
            hi = pltpu.make_async_copy(src.at[pl.ds(7, 1), pl.ds(r, 8), cs], dst.at[pl.ds(7, 1), pl.ds(r, 8), cs],
                                       sem.at[bank, j & (_RING - 1), 2 * p + 1])
            out.append((lo, hi))
        return out

    wm_step = functools.partial(w_step, wm_hbm, wm_buf, 0, 4, 6 * D // 4)
    wq_step = functools.partial(w_step, wq_hbm, wq_buf, 1, 8, _HQ * _DH // 8)
    wo_step = functools.partial(w_step, wo_hbm, wo_buf, 0, 1, D)
    N_WM, N_WQ, N_WO = 16, 32, 32

    def start(step):
        for lo, hi in step:
            lo.start(priority=1)
            hi.start(priority=0)

    def advance(wait_step, start_step):
        for p, (lo, hi) in enumerate(wait_step):
            lo.wait()
            if start_step is not None:
                start_step[p][0].start(priority=1)
                start_step[p][1].start(priority=0)
            hi.wait()

    def loop(n, body):
        def f(i, c):
            body(i)
            return c
        lax.fori_loop(0, n, f, 0)

    def phase(cur, n, nxt, compute, nbody, spb):
        def body(i):
            for t in range(spb):
                j = i * spb + t
                advance(cur(j), cur(j + _LA))
                if t == 0:
                    compute(i)
        if nbody:
            loop(nbody, body)
        done = nbody * spb
        if n - _LA > done:
            loop(n - _LA - done, lambda i: advance(cur(done + i), cur(done + i + _LA)))
        loop(_LA, lambda i: advance(cur(n - _LA + i), None if nxt is None else nxt(i)))

    cx = pltpu.make_async_copy(x_hbm, x_buf, sem2.at[0])
    cc = pltpu.make_async_copy(c_hbm, c_buf, sem2.at[1])
    for i in range(_LA):
        start(wm_step(i))
    cx.start()
    cc.start()
    phase(wm_step, N_WM, wq_step, None, 0, 0)

    cc.wait()
    cx.wait()
    c = c_buf[...].astype(_F32)
    h_ref[...] = c * _sigmoid(c)

    MB = mod_ref.shape[0]
    MW = mod_ref.shape[2]

    def mod_block(i):
        w = wm_buf[:, :, pl.ds(pl.multiple_of(i * MW, 128), MW)].reshape(D, MW)
        mod_ref[i] = jnp.dot(h_ref[...].astype(_BF16), w, preferred_element_type=_F32)

    phase(wq_step, N_WQ, functools.partial(k_step, 0), mod_block, MB, 2)

    def mod(k):
        per = D // MW
        return jnp.concatenate([mod_ref[k * per + t] for t in range(per)], axis=-1)

    def load_x():
        return x_buf[...].astype(_F32)

    h_ref[...] = _layernorm(load_x()) * (1.0 + mod(1)) + mod(0)

    def q_block(i):
        w = wq_buf[:, :, pl.ds(pl.multiple_of(i * 4 * _DH, 128), 4 * _DH)].reshape(D, 4 * _DH)
        q = jnp.dot(h_ref[...].astype(_BF16), w, preferred_element_type=_F32)
        for t in range(4):
            q_ref[4 * i + t] = q[:, t * _DH:(t + 1) * _DH]

    phase(functools.partial(k_step, 0), NSTEP, functools.partial(v_step, 0), q_block, 8, 3)

    def unit_bh(g, u):
        return g >> (GPB.bit_length() - 1), (g & (GPB - 1)) * _S + u

    def qk(g, i):
        for t in range(2):
            u = 2 * i + t
            b, h = unit_bh(g, u)
            q = q_ref[h, pl.ds(b, 1), :].astype(_BF16)
            s_ref[pl.ds(u, 1), :] = lax.dot_general(q, kbuf[u], _NT, preferred_element_type=_F32)

    def softmax():
        s = s_ref[...] * scale
        m = jnp.max(s, axis=-1, keepdims=True)
        p = jnp.exp(s - m)
        s_ref[...] = p * (1.0 / jnp.sum(p, axis=-1, keepdims=True))

    def pv(g, i):
        for t in range(2):
            u = 2 * i + t
            b, h = unit_bh(g, u)
            p = s_ref[pl.ds(u, 1), :].astype(_BF16)
            o_ref[h, pl.ds(b, 1), :] = jnp.dot(p, vbuf[u], preferred_element_type=_F32)

    def group(g):
        phase(functools.partial(v_step, g), NSTEP, functools.partial(k_step, g + 1),
              functools.partial(qk, g), 8, 3)
        softmax()
        phase(functools.partial(k_step, g + 1), NSTEP, functools.partial(v_step, g + 1),
              functools.partial(pv, g), 8, 3)

    loop(NG - 1, group)
    phase(functools.partial(v_step, NG - 1), NSTEP, wo_step, functools.partial(qk, NG - 1), 8, 3)
    softmax()

    queue = [([lo], hi) for j in range(N_WO) for lo, hi in wo_step(j)]

    FH = F // 2
    NFB = FH // 64
    blocks = [(NFB * 64, FH - NFB * 64)] + [(64 * t, 64) for t in range(NFB)]

    def add_group(a_src, a_dst, ra, b_src, b_dst, rb):
        si = 2 + 3 * (len(queue) % _FRING)
        ra, rb = pl.ds(ra, _FP), pl.ds(rb, _FP)
        queue.append(([pltpu.make_async_copy(a_src.at[:, ra], a_dst.at[:, ra], sem2.at[si]),
                       pltpu.make_async_copy(b_src.at[0, rb], b_dst.at[0, rb], sem2.at[si + 1])],
                      pltpu.make_async_copy(b_src.at[1, rb], b_dst.at[1, rb], sem2.at[si + 2])))

    gu_ready = []
    for r, n in blocks:
        for r0 in range(r, r + n, _FP):
            add_group(wg_hbm, wg_buf, r0, wu_hbm, wu_buf, r0)
        gu_ready.append(len(queue))
    rs = pl.ds(blocks[0][0], blocks[0][1])
    si = 2 + 3 * (len(queue) % _FRING)
    queue.append(([pltpu.make_async_copy(wd_hbm.at[0, rs], wd_buf.at[0, rs], sem2.at[si])],
                  pltpu.make_async_copy(wd_hbm.at[1, rs], wd_buf.at[1, rs], sem2.at[si + 1])))
    d_ready = []
    for t in range(NFB // 2):
        for r0 in range(64 * t, 64 * t + 64, _FP):
            add_group(wd_hbm, wd_buf, r0, wd_hbm, wd_buf, r0 + 64 * (NFB // 2))
        d_ready.append(len(queue))
    state = dict(started=2 * _LA, waited=0)

    def pump(upto):
        while state["waited"] < min(upto, len(queue)):
            los, hi = queue[state["waited"]]
            for lo in los:
                lo.wait()
            if state["started"] < len(queue):
                nlos, nhi = queue[state["started"]]
                for lo in nlos:
                    lo.start(priority=1)
                nhi.start(priority=0)
                state["started"] += 1
            hi.wait()
            state["waited"] += 1

    for i in range(8):
        pump(3 * i + 2)
        pv(NG - 1, i)

    attn = jnp.zeros((B, D), _F32)
    for t in range(4):
        pump(max(16 * (t + 1), state["waited"] + 4))
        o = jnp.concatenate([o_ref[4 * i + t] for i in range(8)], axis=-1).astype(_BF16)
        w = wo_buf[:, t * _DH:(t + 1) * _DH, :].reshape(8 * _DH, D)
        attn = attn + jnp.dot(o, w, preferred_element_type=_F32)
    pump(state["waited"] + 3)

    x1 = load_x() + mod(2) * attn
    h2 = (_layernorm(x1) * (1.0 + mod(4)) + mod(3)).astype(_BF16)

    def rows_of(buf, r, n):
        return buf[:, r:r + n, :].reshape(2 * n, D)

    hh = []
    for t, (r, n) in enumerate(blocks):
        pump(max(gu_ready[t], state["waited"] + 3))
        gate = lax.dot_general(h2, rows_of(wg_buf, r, n), _NT, preferred_element_type=_F32)
        up = lax.dot_general(h2, rows_of(wu_buf, r, n), _NT, preferred_element_type=_F32)
        hh.append((_sigmoid(gate) * up).astype(_BF16))
    y = jnp.zeros((B, D), _F32)
    for t in range(NFB // 2):
        pump(d_ready[t])
        for k in ([0] if t == 0 else []) + [1 + t, 1 + t + NFB // 2]:
            y = y + jnp.dot(hh[k], rows_of(wd_buf, *blocks[k]), preferred_element_type=_F32)
    out_ref[...] = (x1 + mod(5) * y).astype(out_ref.dtype)


@jax.jit
def pallas_adaLN_cond__sliding_block_cached__glu_gated_glu__decode_kernel(
    A_x: jax.Array,
    A_k_cache: jax.Array,
    A_v_cache: jax.Array,
    A_wq: jax.Array,
    A_wo: jax.Array,
    B_x: jax.Array,
    B_w_gate: jax.Array,
    B_w_up: jax.Array,
    B_w_down: jax.Array,
    c: jax.Array,
    w_mod: jax.Array,
):
    del B_x
    B, Sq, D = A_x.shape
    Hkv, Sk = A_k_cache.shape[1], A_k_cache.shape[2]
    F = B_w_gate.shape[1]
    assert Sq == 1 and Hkv == _HQ and A_k_cache.shape[3] == _DH
    W = min(4096, max(256, Sk // 4))
    NG = B * _HQ // _S

    k = A_k_cache.reshape(NG, _S, Sk, _DH)
    v = A_v_cache.reshape(NG, _S, Sk, _DH)
    wq = A_wq.reshape(8, D // 8, _HQ * _DH)
    wo = A_wo.reshape(8, _HQ * _DH // 8, D)
    wm = w_mod.reshape(8, D // 8, 6 * D)
    x = A_x.reshape(B, D)
    wg = B_w_gate.T.reshape(2, F // 2, D)
    wu = B_w_up.T.reshape(2, F // 2, D)
    wd = B_w_down.reshape(2, F // 2, D)

    any_spec = pl.BlockSpec(memory_space=pl.ANY)
    out = pl.pallas_call(
        functools.partial(_kernel, B=B, D=D, F=F, Sk=Sk, W=W),
        out_shape=jax.ShapeDtypeStruct(x.shape, x.dtype),
        in_specs=[any_spec] * 10,
        out_specs=pl.BlockSpec(memory_space=pltpu.VMEM),
        scratch_shapes=[
            pltpu.VMEM((_S, W, _DH), _BF16),
            pltpu.VMEM((_S, W, _DH), _BF16),
            pltpu.VMEM(wm.shape, _BF16),
            pltpu.VMEM(wq.shape, _BF16),
            pltpu.VMEM(wo.shape, _BF16),
            pltpu.VMEM(wg.shape, _BF16),
            pltpu.VMEM(wu.shape, _BF16),
            pltpu.VMEM(wd.shape, _BF16),
            pltpu.VMEM(x.shape, _BF16),
            pltpu.VMEM(c.shape, _BF16),
            pltpu.VMEM((12, B, 6 * D // 12), _F32),
            pltpu.VMEM((_HQ, B, _DH), _F32),
            pltpu.VMEM((_HQ, B, _DH), _F32),
            pltpu.VMEM((_S, W), _F32),
            pltpu.VMEM((B, D), _F32),
            pltpu.SemaphoreType.DMA((2, _RING, 4)),
            pltpu.SemaphoreType.DMA((2 + 3 * _FRING,)),
        ],
        compiler_params=pltpu.CompilerParams(
            vmem_limit_bytes=64 * 1024 * 1024,
            disable_bounds_checks=True,
            disable_semaphore_checks=True,
        ),
    )(x, k, v, wq, wo, wg, wu, wd, c, wm)
    return out.reshape(A_x.shape)
```

```python
import functools

import jax
import jax.numpy as jnp
from jax import lax
import jax.experimental.pallas as pl
import jax.experimental.pallas.tpu as pltpu

_F32 = jnp.float32
_BF16 = jnp.bfloat16
_NT = (((1,), (1,)), ((), ()))

_HQ = 32
_DH = 128
_EPS = 1e-5
_S = 16
_RING = 32
_FP = 16

_CFG = dict(
    R=32,
    SHIFT=8,
    ROT=1,
    LA1=18,
    LA0=10,
    PPB=5,
)


def _layernorm(x):
    m = jnp.mean(x, axis=-1, keepdims=True)
    xc = x - m
    v = jnp.mean(xc * xc, axis=-1, keepdims=True)
    return xc * lax.rsqrt(v + _EPS)


class _Phase:
    def __init__(self, n, lo, hi, head=None, tail=None):
        self.n, self.lo, self.hi = n, lo, hi
        self.head = head or (lambda: [])
        self.tail = tail or (lambda: [])


def _kernel(x_hbm, k_hbm, v_hbm, wq_hbm, wo_hbm, wg_hbm, wu_hbm, wd_hbm, c_hbm, wm_hbm,
            out_ref,
            kbuf, vbuf, wm_buf, wq_buf, wo_buf, wg_buf, wu_buf, wd_buf, x_buf, c_buf,
            mod_ref, q_ref, o_ref, s_ref, h_ref, sem, esem, fsem,
            *, B, D, F, Sk, W):
    R, SHIFT, ROT, LA1, LA0, PPB = (_CFG[k] for k in ("R", "SHIFT", "ROT", "LA1", "LA0", "PPB"))
    NG = k_hbm.shape[0]
    GPB = _HQ // _S
    scale = _DH ** -0.5
    copy = pltpu.make_async_copy

    PPS = R // 16
    NLO, NHI = (_S - 2) // PPS, 2 // PPS
    NSLAB = (W - SHIFT) // R
    TAIL0 = SHIFT + NSLAB * R

    def kv_phase(src, dst, bank, g):
        g_hi = (g + ROT) & (NG - 1)

        def piece(gg, s, r, n, sm):
            return copy(src.at[gg, s, pl.ds(Sk - W + r, n), :], dst.at[s, pl.ds(r, n), :], sm)

        def row(e):
            return pl.multiple_of(SHIFT + (e >> (PPS - 1)) * R, 8)

        def lo(e):
            return piece(g, pl.ds(2 + (e & (PPS - 1)) * NLO, NLO), row(e), R, sem.at[bank, e & (_RING - 1), 0])

        def hi(e):
            return piece(g_hi, pl.ds((e & (PPS - 1)) * NHI, NHI), row(e), R, sem.at[bank, e & (_RING - 1), 1])

        def edge(r, n, k):
            if n == 0:
                return []
            return [piece(g, pl.ds(2, _S - 2), r, n, esem.at[bank, k]),
                    piece(g_hi, pl.ds(0, 2), r, n, esem.at[bank, k + 1])]

        return _Phase(NSLAB * PPS, lo, hi, lambda: edge(0, SHIFT, 0), lambda: edge(TAIL0, W - TAIL0, 2))

    k_phase = functools.partial(kv_phase, k_hbm, kbuf, 0)
    v_phase = functools.partial(kv_phase, v_hbm, vbuf, 1)

    def w_phase(src, dst, bank, ncb):
        cw = src.shape[2] // ncb

        def piece(s, e, k):
            r = pl.ds(pl.multiple_of((e >> (ncb.bit_length() - 1)) * 8, 8), 8)
            cs = slice(None) if ncb == 1 else pl.ds(pl.multiple_of((e & (ncb - 1)) * cw, 128), cw)
            return copy(src.at[s, r, cs], dst.at[s, r, cs], sem.at[bank, e & (_RING - 1), k])

        return _Phase(src.shape[1] // 8 * ncb, lambda e: piece(pl.ds(0, 7), e, 0), lambda e: piece(pl.ds(7, 1), e, 1))

    wm_phase = w_phase(wm_hbm, wm_buf, 0, 4)
    wq_phase = w_phase(wq_hbm, wq_buf, 1, 8)
    wo_phase = w_phase(wo_hbm, wo_buf, 0, 1)

    def loop(n, body):
        def f(i, c):
            body(i)
            return c
        if n > 0:
            lax.fori_loop(0, n, f, 0)

    def run(cur, nxt, compute=None, nbody=0, ppb=0):
        n = cur.n

        def advance(e, lo_next, hi_next):
            cur.lo(e).wait()
            lo_next.start(priority=1)
            hi_next.start(priority=0)
            cur.hi(e).wait()

        def body(i):
            for t in range(ppb):
                e = i * ppb + t
                advance(e, cur.lo(e + LA1), cur.hi(e + LA0))
                if t == 0:
                    compute(i)

        for cp in cur.head():
            cp.wait()
        loop(nbody, body)
        a = nbody * ppb
        assert a <= n - LA1
        loop(n - LA1 - a, lambda i: advance(a + i, cur.lo(a + i + LA1), cur.hi(a + i + LA0)))
        for cp in cur.tail() + nxt.head():
            cp.start(priority=1)
        b = n - LA1
        loop(LA1 - LA0, lambda i: advance(b + i, nxt.lo(i), cur.hi(b + i + LA0)))
        c0 = n - LA0
        loop(LA0, lambda i: advance(c0 + i, nxt.lo(LA1 - LA0 + i), nxt.hi(i)))
        for cp in cur.tail():
            cp.wait()

    for e in range(LA1):
        wm_phase.lo(e).start(priority=1)
        if e < LA0:
            wm_phase.hi(e).start(priority=0)
    cx = copy(x_hbm, x_buf, fsem.at[0])
    cc = copy(c_hbm, c_buf, fsem.at[1])
    cx.start()
    cc.start()
    run(wm_phase, wq_phase)

    cc.wait()
    cx.wait()
    c = c_buf[...].astype(_F32)
    h_ref[...] = c * jax.nn.sigmoid(c)

    MB, MW = mod_ref.shape[0], mod_ref.shape[2]

    def mod_block(i):
        w = wm_buf[:, :, pl.ds(pl.multiple_of(i * MW, 128), MW)].reshape(D, MW)
        mod_ref[i] = jnp.dot(h_ref[...].astype(_BF16), w, preferred_element_type=_F32)

    run(wq_phase, k_phase(0), mod_block, MB, (wq_phase.n - LA1) // MB)

    def mod(k):
        per = D // MW
        return jnp.concatenate([mod_ref[k * per + t] for t in range(per)], axis=-1)

    h_ref[...] = _layernorm(x_buf[...].astype(_F32)) * (1.0 + mod(1)) + mod(0)

    def q_block(i):
        w = wq_buf[:, :, pl.ds(pl.multiple_of(i * 4 * _DH, 128), 4 * _DH)].reshape(D, 4 * _DH)
        q = jnp.dot(h_ref[...].astype(_BF16), w, preferred_element_type=_F32)
        for t in range(4):
            q_ref[4 * i + t] = q[:, t * _DH:(t + 1) * _DH]

    run(k_phase(0), v_phase(0), q_block, _HQ // 4, PPB)

    def units(g, i):
        if isinstance(i, int):
            gg = (g + (ROT if i == 0 else 0)) & (NG - 1)
        else:
            gg = (g + jnp.where(i == 0, ROT, 0)) & (NG - 1)
        b = gg >> (GPB.bit_length() - 1)
        return [(2 * i + t, b, (gg & (GPB - 1)) * _S + 2 * i + t) for t in range(2)]

    def qk(g, i):
        for u, b, h in units(g, i):
            q = q_ref[h, pl.ds(b, 1), :].astype(_BF16)
            s_ref[pl.ds(u, 1), :] = lax.dot_general(q, kbuf[u], _NT, preferred_element_type=_F32)

    def softmax():
        s = s_ref[...] * scale
        m = jnp.max(s, axis=-1, keepdims=True)
        p = jnp.exp(s - m)
        s_ref[...] = p * (1.0 / jnp.sum(p, axis=-1, keepdims=True))

    def pv(g, i):
        for u, b, h in units(g, i):
            p = s_ref[pl.ds(u, 1), :].astype(_BF16)
            o_ref[h, pl.ds(b, 1), :] = jnp.dot(p, vbuf[u], preferred_element_type=_F32)

    def group(g):
        run(v_phase(g), k_phase(g + 1), functools.partial(qk, g), _S // 2, PPB)
        softmax()
        run(k_phase(g + 1), v_phase(g + 1), functools.partial(pv, g), _S // 2, PPB)

    loop(NG - 1, group)
    run(v_phase(NG - 1), wo_phase, functools.partial(qk, NG - 1), _S // 2, PPB)
    softmax()

    queue = [([wo_phase.lo(e)], wo_phase.hi(e)) for e in range(wo_phase.n)]

    FH = F // 2
    NFB = FH // 64
    blocks = [(NFB * 64, FH - NFB * 64)] + [(64 * t, 64) for t in range(NFB)]

    def add_group(a_src, a_dst, ra, b_src, b_dst, rb):
        si = 2 + 3 * (len(queue) % _RING)
        ra, rb = pl.ds(ra, _FP), pl.ds(rb, _FP)
        queue.append(([copy(a_src.at[:, ra], a_dst.at[:, ra], fsem.at[si]),
                       copy(b_src.at[0, rb], b_dst.at[0, rb], fsem.at[si + 1])],
                      copy(b_src.at[1, rb], b_dst.at[1, rb], fsem.at[si + 2])))

    gu_ready = []
    for r, n in blocks:
        for r0 in range(r, r + n, _FP):
            add_group(wg_hbm, wg_buf, r0, wu_hbm, wu_buf, r0)
        gu_ready.append(len(queue))
    rs = pl.ds(blocks[0][0], blocks[0][1])
    si = 2 + 3 * (len(queue) % _RING)
    queue.append(([copy(wd_hbm.at[0, rs], wd_buf.at[0, rs], fsem.at[si])],
                  copy(wd_hbm.at[1, rs], wd_buf.at[1, rs], fsem.at[si + 1])))
    d_ready = []
    for t in range(NFB // 2):
        for r0 in range(64 * t, 64 * t + 64, _FP):
            add_group(wd_hbm, wd_buf, r0, wd_hbm, wd_buf, r0 + 64 * (NFB // 2))
        d_ready.append(len(queue))
    waited = [0]

    def pump(upto):
        while waited[0] < min(upto, len(queue)):
            e = waited[0]
            for cp in queue[e][0]:
                cp.wait()
            if e + LA1 < len(queue):
                for cp in queue[e + LA1][0]:
                    cp.start(priority=1)
            if e + LA0 < len(queue):
                queue[e + LA0][1].start(priority=0)
            queue[e][1].wait()
            waited[0] += 1

    for i in range(_S // 2):
        pump(3 * i + 2)
        pv(NG - 1, i)

    attn = jnp.zeros((B, D), _F32)
    for t in range(4):
        pump(max(16 * (t + 1), waited[0] + 4))
        o = jnp.concatenate([o_ref[4 * i + t] for i in range(8)], axis=-1).astype(_BF16)
        w = wo_buf[:, t * _DH:(t + 1) * _DH, :].reshape(8 * _DH, D)
        attn = attn + jnp.dot(o, w, preferred_element_type=_F32)
    pump(waited[0] + 3)

    x1 = x_buf[...].astype(_F32) + mod(2) * attn
    h2 = (_layernorm(x1) * (1.0 + mod(4)) + mod(3)).astype(_BF16)

    def rows_of(buf, r, n):
        return buf[:, r:r + n, :].reshape(2 * n, D)

    hh = []
    for t, (r, n) in enumerate(blocks):
        pump(max(gu_ready[t], waited[0] + 3))
        gate = lax.dot_general(h2, rows_of(wg_buf, r, n), _NT, preferred_element_type=_F32)
        up = lax.dot_general(h2, rows_of(wu_buf, r, n), _NT, preferred_element_type=_F32)
        hh.append((jax.nn.sigmoid(gate) * up).astype(_BF16))
    y = jnp.zeros((B, D), _F32)
    for t in range(NFB // 2):
        pump(d_ready[t])
        for k in ([0] if t == 0 else []) + [1 + t, 1 + t + NFB // 2]:
            y = y + jnp.dot(hh[k], rows_of(wd_buf, *blocks[k]), preferred_element_type=_F32)
    out_ref[...] = (x1 + mod(5) * y).astype(out_ref.dtype)


@jax.jit
def pallas_adaLN_cond__sliding_block_cached__glu_gated_glu__decode_kernel(
    A_x: jax.Array,
    A_k_cache: jax.Array,
    A_v_cache: jax.Array,
    A_wq: jax.Array,
    A_wo: jax.Array,
    B_x: jax.Array,
    B_w_gate: jax.Array,
    B_w_up: jax.Array,
    B_w_down: jax.Array,
    c: jax.Array,
    w_mod: jax.Array,
):
    del B_x
    B, Sq, D = A_x.shape
    Hkv, Sk = A_k_cache.shape[1], A_k_cache.shape[2]
    F = B_w_gate.shape[1]
    assert Sq == 1 and Hkv == _HQ and A_k_cache.shape[3] == _DH
    W = min(4096, max(256, Sk // 4))
    NG = B * _HQ // _S

    x = A_x.reshape(B, D)
    k = A_k_cache.reshape(NG, _S, Sk, _DH)
    v = A_v_cache.reshape(NG, _S, Sk, _DH)
    wq = A_wq.reshape(8, D // 8, _HQ * _DH)
    wo = A_wo.reshape(8, _HQ * _DH // 8, D)
    wm = w_mod.reshape(8, D // 8, 6 * D)
    wg = B_w_gate.T.reshape(2, F // 2, D)
    wu = B_w_up.T.reshape(2, F // 2, D)
    wd = B_w_down.reshape(2, F // 2, D)

    any_spec = pl.BlockSpec(memory_space=pl.ANY)
    out = pl.pallas_call(
        functools.partial(_kernel, B=B, D=D, F=F, Sk=Sk, W=W),
        out_shape=jax.ShapeDtypeStruct(x.shape, x.dtype),
        in_specs=[any_spec] * 10,
        out_specs=pl.BlockSpec(memory_space=pltpu.VMEM),
        scratch_shapes=[
            pltpu.VMEM((_S, W, _DH), _BF16),
            pltpu.VMEM((_S, W, _DH), _BF16),
            pltpu.VMEM(wm.shape, _BF16),
            pltpu.VMEM(wq.shape, _BF16),
            pltpu.VMEM(wo.shape, _BF16),
            pltpu.VMEM(wg.shape, _BF16),
            pltpu.VMEM(wu.shape, _BF16),
            pltpu.VMEM(wd.shape, _BF16),
            pltpu.VMEM(x.shape, _BF16),
            pltpu.VMEM(c.shape, _BF16),
            pltpu.VMEM((12, B, 6 * D // 12), _F32),
            pltpu.VMEM((_HQ, B, _DH), _F32),
            pltpu.VMEM((_HQ, B, _DH), _F32),
            pltpu.VMEM((_S, W), _F32),
            pltpu.VMEM((B, D), _F32),
            pltpu.SemaphoreType.DMA((2, _RING, 2)),
            pltpu.SemaphoreType.DMA((2, 4)),
            pltpu.SemaphoreType.DMA((2 + 3 * _RING,)),
        ],
        compiler_params=pltpu.CompilerParams(
            vmem_limit_bytes=64 * 1024 * 1024,
            disable_bounds_checks=_CFG.get("FAST", True),
            disable_semaphore_checks=_CFG.get("FAST", True),
        ),
    )(x, k, v, wq, wo, wg, wu, wd, c, wm)
    return out.reshape(A_x.shape)
```

```python
import functools

import jax
import jax.numpy as jnp
from jax import lax
import jax.experimental.pallas as pl
import jax.experimental.pallas.tpu as pltpu

_F32 = jnp.float32
_BF16 = jnp.bfloat16
_NT = (((1,), (1,)), ((), ()))

_HQ = 32
_DH = 128
_EPS = 1e-5
_S = 16
_RING = 32
_FP = 16

_CFG = dict(
    R=32,
    SHIFT=8,
    ROT=1,
    LA1=18,
    LA0=9,
    PPB=5,
    CUTS=(-3, -1),
    LAG=16,
)


def _layernorm(x):
    m = jnp.mean(x, axis=-1, keepdims=True)
    xc = x - m
    v = jnp.mean(xc * xc, axis=-1, keepdims=True)
    return xc * lax.rsqrt(v + _EPS)


class _Phase:
    def __init__(self, n, pair, head=None, tail=None):
        self.pair, self.head, self.tail = pair, head, tail
        self.first = 0 if head is None else 1
        self.n = n + self.first + (0 if tail is None else 1)

    def kind(self, t):
        if self.head is not None and t == 0:
            return "head"
        if self.tail is not None and t == self.n - 1:
            return "tail"
        return "pair"

    def at(self, t0, i, cls):
        kind = self.kind(t0)
        if kind == "pair":
            return self.pair(t0 - self.first + i, cls)
        return self.head(cls) if kind == "head" else self.tail(cls)


def _kernel(x_hbm, k_hbm, v_hbm, wq_hbm, wo_hbm, wg_hbm, wu_hbm, wd_hbm, c_hbm, wm_hbm,
            out_ref,
            kbuf, vbuf, wm_buf, wq_buf, wo_buf, wg_buf, wu_buf, wd_buf, x_buf, c_buf,
            mod_ref, q_ref, o_ref, s_ref, h_ref, sem, esem, fsem,
            *, B, D, F, Sk, W):
    R, SHIFT, ROT, LA1, LA0, PPB = (_CFG[k] for k in ("R", "SHIFT", "ROT", "LA1", "LA0", "PPB"))
    NG = k_hbm.shape[0]
    GPB = _HQ // _S
    scale = _DH ** -0.5
    copy = pltpu.make_async_copy

    PPS = R // 16
    NLO, NHI = (_S - 2) // PPS, 2 // PPS
    NSLAB = (W - SHIFT) // R
    TAIL0 = SHIFT + NSLAB * R

    def kv_phase(src, dst, bank, g):
        g_of = ((g + ROT) & (NG - 1), g)

        def piece(cls, s, r, n, sm):
            return copy(src.at[g_of[cls], s, pl.ds(Sk - W + r, n), :], dst.at[s, pl.ds(r, n), :], sm)

        def pair(e, cls):
            r = pl.multiple_of(SHIFT + (e >> (PPS - 1)) * R, 8)
            p = e & (PPS - 1)
            s = pl.ds(2 + p * NLO, NLO) if cls else pl.ds(p * NHI, NHI)
            return piece(cls, s, r, R, sem.at[bank, e & (_RING - 1), cls])

        def edge(r, n, k):
            if n == 0:
                return None
            return lambda cls: piece(cls, pl.ds(2, _S - 2) if cls else pl.ds(0, 2), r, n, esem.at[bank, k + cls])

        return _Phase(NSLAB * PPS, pair, edge(0, SHIFT, 0), edge(TAIL0, W - TAIL0, 2))

    k_phase = functools.partial(kv_phase, k_hbm, kbuf, 0)
    v_phase = functools.partial(kv_phase, v_hbm, vbuf, 1)

    def w_phase(src, dst, bank, ncb):
        cw = src.shape[2] // ncb

        def pair(e, cls):
            s = pl.ds(0, 7) if cls else pl.ds(7, 1)
            r = pl.ds(pl.multiple_of((e >> (ncb.bit_length() - 1)) * 8, 8), 8)
            cs = slice(None) if ncb == 1 else pl.ds(pl.multiple_of((e & (ncb - 1)) * cw, 128), cw)
            return copy(src.at[s, r, cs], dst.at[s, r, cs], sem.at[bank, e & (_RING - 1), cls])

        return _Phase(src.shape[1] // 8 * ncb, pair)

    wm_phase = w_phase(wm_hbm, wm_buf, 0, 4)
    wq_phase = w_phase(wq_hbm, wq_buf, 1, 8)
    wo_phase = w_phase(wo_hbm, wo_buf, 0, 1)

    def loop(n, body):
        def f(i, c):
            body(i)
            return c
        if n == 1:
            body(0)
        elif n > 1:
            lax.fori_loop(0, n, f, 0)

    def run(cur, nxt, compute=None, nbody=0, ppb=0):
        def ahead(t):
            return (cur, t) if t < cur.n else (nxt, t - cur.n)

        def tick(t0, i):
            (p1, t1), (p0, t2) = ahead(t0 + LA1), ahead(t0 + LA0)
            cur.at(t0, i, 1).wait()
            p1.at(t1, i, 1).start(priority=1)
            p0.at(t2, i, 0).start(priority=0)
            cur.at(t0, i, 0).wait()

        def signature(t):
            return [cur.kind(t)] + [(p is cur, p.kind(u)) for p, u in (ahead(t + LA1), ahead(t + LA0))]

        t = 0
        while t < cur.n:
            n = 1
            while t + n < cur.n and signature(t + n) == signature(t):
                n += 1
            if t == cur.first and nbody:
                assert nbody * ppb <= n and t + n + LA1 <= cur.n
                n = nbody * ppb

                def body(i, t=t):
                    for k in range(ppb):
                        tick(t, i * ppb + k)
                        if k == 0:
                            compute(i)
                loop(nbody, body)
            else:
                loop(n, functools.partial(tick, t))
            t += n

    for e in range(LA1):
        wm_phase.pair(e, 1).start(priority=1)
        if e < LA0:
            wm_phase.pair(e, 0).start(priority=0)
    cx = copy(x_hbm, x_buf, fsem.at[0])
    cc = copy(c_hbm, c_buf, fsem.at[1])
    cx.start()
    cc.start()
    run(wm_phase, wq_phase)

    cc.wait()
    cx.wait()
    c = c_buf[...].astype(_F32)
    h_ref[...] = c * jax.nn.sigmoid(c)

    MB, MW = mod_ref.shape[0], mod_ref.shape[2]

    def mod_block(i):
        w = wm_buf[:, :, pl.ds(pl.multiple_of(i * MW, 128), MW)].reshape(D, MW)
        mod_ref[i] = jnp.dot(h_ref[...].astype(_BF16), w, preferred_element_type=_F32)

    run(wq_phase, k_phase(0), mod_block, MB, (wq_phase.n - LA1) // MB)

    def mod(k):
        per = D // MW
        return jnp.concatenate([mod_ref[k * per + t] for t in range(per)], axis=-1)

    h_ref[...] = _layernorm(x_buf[...].astype(_F32)) * (1.0 + mod(1)) + mod(0)

    def q_block(i):
        w = wq_buf[:, :, pl.ds(pl.multiple_of(i * 4 * _DH, 128), 4 * _DH)].reshape(D, 4 * _DH)
        q = jnp.dot(h_ref[...].astype(_BF16), w, preferred_element_type=_F32)
        for t in range(4):
            q_ref[4 * i + t] = q[:, t * _DH:(t + 1) * _DH]

    run(k_phase(0), v_phase(0), q_block, _HQ // 4, PPB)

    def units(g, i):
        if isinstance(i, int):
            gg = (g + (ROT if i == 0 else 0)) & (NG - 1)
        else:
            gg = (g + jnp.where(i == 0, ROT, 0)) & (NG - 1)
        b = gg >> (GPB.bit_length() - 1)
        return [(2 * i + t, b, (gg & (GPB - 1)) * _S + 2 * i + t) for t in range(2)]

    def qk(g, i):
        for u, b, h in units(g, i):
            q = q_ref[h, pl.ds(b, 1), :].astype(_BF16)
            s_ref[pl.ds(u, 1), :] = lax.dot_general(q, kbuf[u], _NT, preferred_element_type=_F32)

    def softmax():
        s = s_ref[...] * scale
        m = jnp.max(s, axis=-1, keepdims=True)
        p = jnp.exp(s - m)
        s_ref[...] = p * (1.0 / jnp.sum(p, axis=-1, keepdims=True))

    def pv(g, i):
        for u, b, h in units(g, i):
            p = s_ref[pl.ds(u, 1), :].astype(_BF16)
            o_ref[h, pl.ds(b, 1), :] = jnp.dot(p, vbuf[u], preferred_element_type=_F32)

    def group(g):
        run(v_phase(g), k_phase(g + 1), functools.partial(qk, g), _S // 2, PPB)
        softmax()
        run(k_phase(g + 1), v_phase(g + 1), functools.partial(pv, g), _S // 2, PPB)

    loop(NG - 1, group)
    run(v_phase(NG - 1), wo_phase, functools.partial(qk, NG - 1), _S // 2, PPB)
    softmax()

    queue = [([wo_phase.pair(e, 1)], wo_phase.pair(e, 0), 4) for e in range(wo_phase.n)]

    FH = F // 2
    NU = FH // _FP
    LAG = _CFG["LAG"]
    blocks = [(r, min(64, FH - r)) for r in range(0, FH, 64)]
    n_wo = len(queue)
    for i in range(NU + LAG):
        parts = []
        if i < NU:
            parts += [(wg_hbm, wg_buf, i), (wu_hbm, wu_buf, i)]
        if i >= LAG:
            parts += [(wd_hbm, wd_buf, i - LAG)]
        si = 2 + 4 * (len(queue) % _RING)
        cps = []
        for k, (src, dst, u) in enumerate(parts):
            rows = pl.ds(u * _FP, _FP)
            for half in ([slice(None)] if k + 1 < len(parts) else [0, 1]):
                cps.append(copy(src.at[half, rows], dst.at[half, rows], fsem.at[si + len(cps)]))
        queue.append((cps[:-1], cps[-1], 2 * len(parts)))
    gu_ready = [n_wo + (r + n) // _FP for r, n in blocks]
    d_ready = [t + LAG for t in gu_ready]
    cum = [0]
    for item in queue:
        cum.append(cum[-1] + item[2])
    waited, started = [0], [LA0, LA1]

    def pump(upto):
        while waited[0] < min(upto, len(queue)):
            e = waited[0]
            for cp in queue[e][0]:
                cp.wait()
            for cls, la in ((1, LA1), (0, LA0)):
                while started[cls] < len(queue) and cum[started[cls]] < cum[e + 1] + 4 * la:
                    assert started[cls] - e < _RING
                    for cp in (queue[started[cls]][0] if cls else [queue[started[cls]][1]]):
                        cp.start(priority=cls)
                    started[cls] += 1
            queue[e][1].wait()
            waited[0] += 1

    for i in range(_S // 2):
        pump(3 * i + 2)
        pv(NG - 1, i)

    attn = jnp.zeros((B, D), _F32)
    for t in range(4):
        pump(max(16 * (t + 1), waited[0] + 4))
        o = jnp.concatenate([o_ref[4 * i + t] for i in range(8)], axis=-1).astype(_BF16)
        w = wo_buf[:, t * _DH:(t + 1) * _DH, :].reshape(8 * _DH, D)
        attn = attn + jnp.dot(o, w, preferred_element_type=_F32)
    pump(waited[0] + 3)

    x1 = x_buf[...].astype(_F32) + mod(2) * attn
    h2 = (_layernorm(x1) * (1.0 + mod(4)) + mod(3)).astype(_BF16)

    def rows_of(buf, r, n):
        return buf[:, r:r + n, :].reshape(2 * n, D)

    hh = []
    y = jnp.zeros((B, D), _F32)
    n_down = 0

    def down(k):
        return jnp.dot(hh[k], rows_of(wd_buf, *blocks[k]), preferred_element_type=_F32)

    for t, (r, n) in enumerate(blocks):
        pump(max(gu_ready[t], waited[0] + 2))
        while n_down < len(hh) and d_ready[n_down] <= waited[0]:
            y = y + down(n_down)
            n_down += 1
        gate = lax.dot_general(h2, rows_of(wg_buf, r, n), _NT, preferred_element_type=_F32)
        up = lax.dot_general(h2, rows_of(wu_buf, r, n), _NT, preferred_element_type=_F32)
        hh.append((jax.nn.sigmoid(gate) * up).astype(_BF16))
    for last in _CFG["CUTS"]:
        last += len(blocks)
        pump(d_ready[last])
        while n_down <= last:
            y = y + down(n_down)
            n_down += 1
    out_ref[...] = (x1 + mod(5) * y).astype(out_ref.dtype)


@jax.jit
def pallas_adaLN_cond__sliding_block_cached__glu_gated_glu__decode_kernel(
    A_x: jax.Array,
    A_k_cache: jax.Array,
    A_v_cache: jax.Array,
    A_wq: jax.Array,
    A_wo: jax.Array,
    B_x: jax.Array,
    B_w_gate: jax.Array,
    B_w_up: jax.Array,
    B_w_down: jax.Array,
    c: jax.Array,
    w_mod: jax.Array,
):
    del B_x
    B, Sq, D = A_x.shape
    Hkv, Sk = A_k_cache.shape[1], A_k_cache.shape[2]
    F = B_w_gate.shape[1]
    assert Sq == 1 and Hkv == _HQ and A_k_cache.shape[3] == _DH
    W = min(4096, max(256, Sk // 4))
    NG = B * _HQ // _S

    x = A_x.reshape(B, D)
    k = A_k_cache.reshape(NG, _S, Sk, _DH)
    v = A_v_cache.reshape(NG, _S, Sk, _DH)
    wq = A_wq.reshape(8, D // 8, _HQ * _DH)
    wo = A_wo.reshape(8, _HQ * _DH // 8, D)
    wm = w_mod.reshape(8, D // 8, 6 * D)
    wg = B_w_gate.T.reshape(2, F // 2, D)
    wu = B_w_up.T.reshape(2, F // 2, D)
    wd = B_w_down.reshape(2, F // 2, D)

    any_spec = pl.BlockSpec(memory_space=pl.ANY)
    out = pl.pallas_call(
        functools.partial(_kernel, B=B, D=D, F=F, Sk=Sk, W=W),
        out_shape=jax.ShapeDtypeStruct(x.shape, x.dtype),
        in_specs=[any_spec] * 10,
        out_specs=pl.BlockSpec(memory_space=pltpu.VMEM),
        scratch_shapes=[
            pltpu.VMEM((_S, W, _DH), _BF16),
            pltpu.VMEM((_S, W, _DH), _BF16),
            pltpu.VMEM(wm.shape, _BF16),
            pltpu.VMEM(wq.shape, _BF16),
            pltpu.VMEM(wo.shape, _BF16),
            pltpu.VMEM(wg.shape, _BF16),
            pltpu.VMEM(wu.shape, _BF16),
            pltpu.VMEM(wd.shape, _BF16),
            pltpu.VMEM(x.shape, _BF16),
            pltpu.VMEM(c.shape, _BF16),
            pltpu.VMEM((12, B, 6 * D // 12), _F32),
            pltpu.VMEM((_HQ, B, _DH), _F32),
            pltpu.VMEM((_HQ, B, _DH), _F32),
            pltpu.VMEM((_S, W), _F32),
            pltpu.VMEM((B, D), _F32),
            pltpu.SemaphoreType.DMA((2, _RING, 2)),
            pltpu.SemaphoreType.DMA((2, 4)),
            pltpu.SemaphoreType.DMA((2 + 4 * _RING,)),
        ],
        compiler_params=pltpu.CompilerParams(
            vmem_limit_bytes=64 * 1024 * 1024,
            disable_bounds_checks=_CFG.get("FAST", True),
            disable_semaphore_checks=_CFG.get("FAST", True),
        ),
    )(x, k, v, wq, wo, wg, wu, wd, c, wm)
    return out.reshape(A_x.shape)
```

```python
import functools

import jax
import jax.numpy as jnp
from jax import lax
import jax.experimental.pallas as pl
import jax.experimental.pallas.tpu as pltpu

_F32 = jnp.float32
_BF16 = jnp.bfloat16
_NT = (((1,), (1,)), ((), ()))

_HQ = 32
_DH = 128
_EPS = 1e-5
_S = 16
_RING = 32
_FRING = 48
_FP = 16

_CFG = dict(
    R=32,
    SHIFT=8,
    ROT=1,
    LA1=18,
    LA0=9,
    PPB=5,
    CUTS=(-3, -1),
    FINE=0,
    KV62=0,
    MERGE=1,
    WHI=1,
    LAG=16,
)


def _layernorm(x):
    m = jnp.mean(x, axis=-1, keepdims=True)
    xc = x - m
    v = jnp.mean(xc * xc, axis=-1, keepdims=True)
    return xc * lax.rsqrt(v + _EPS)


class _Phase:
    def __init__(self, n, pair, head=None, tail=None, hi_total=None):
        self.pair, self.head, self.tail, self.hi_total = pair, head, tail, hi_total
        self.first = 0 if head is None else 1
        self.n = n + self.first + (0 if tail is None else 1)

    def kind(self, t):
        if self.head is not None and t == 0:
            return "head"
        if self.tail is not None and t == self.n - 1:
            return "tail"
        return "pair"

    def at(self, t0, i, cls):
        kind = self.kind(t0)
        if kind == "pair":
            return self.pair(t0 - self.first + i, cls)
        return self.head(cls) if kind == "head" else self.tail(cls)


def _kernel(x_hbm, k_hbm, v_hbm, wq_hbm, wo_hbm, wg_hbm, wu_hbm, wd_hbm, c_hbm, wm_hbm,
            out_ref,
            kbuf, vbuf, wm_buf, wq_buf, wo_buf, wg_buf, wu_buf, wd_buf, x_buf, c_buf,
            mod_ref, q_ref, o_ref, s_ref, h_ref, sem, esem, fsem,
            *, B, D, F, Sk, W):
    R, SHIFT, ROT, LA1, LA0, PPB = (_CFG[k] for k in ("R", "SHIFT", "ROT", "LA1", "LA0", "PPB"))
    NG = k_hbm.shape[0]
    GPB = _HQ // _S
    scale = _DH ** -0.5
    copy = pltpu.make_async_copy

    NSLAB = (W - SHIFT) // R
    TAIL0 = SHIFT + NSLAB * R

    def kv_phase(src, dst, bank, g):
        g_rot = (g + ROT) & (NG - 1)

        def piece(gg, s, r, n, sm):
            return copy(src.at[gg, s, pl.ds(Sk - W + r, n), :], dst.at[s, pl.ds(r, n), :], sm)

        def pair(e, cls):
            r = pl.multiple_of(SHIFT + (e >> 1) * R, 8)
            p = e & 1
            sm = sem.at[bank, e & (_RING - 1), cls] if cls or not _CFG["MERGE"] else esem.at[bank, 4 + p]
            if _CFG["KV62"]:
                if cls:
                    return piece(g, pl.ds(2 + 6 * p, 6), r, R, sm)
                return piece((g + ROT * (1 - p)) & (NG - 1), pl.ds(14 * p, 2), r, R, sm)
            if cls:
                return piece(g, pl.ds(2 + 7 * p, 7), r, R, sm)
            return piece(g_rot, pl.ds(p, 1), r, R, sm)

        def edge(r, n, k):
            if n == 0:
                return None
            return lambda cls: (piece(g, pl.ds(2, _S - 2), r, n, esem.at[bank, k + 1]) if cls else
                                piece(g_rot, pl.ds(0, 2), r, n, esem.at[bank, k]))

        def hi_total():
            rows = pl.ds(SHIFT, NSLAB * R)
            views = [dst.at[pl.ds(14 * p, 2) if _CFG["KV62"] else pl.ds(p, 1), rows, :] for p in range(2)]
            return [copy(v, v, esem.at[bank, 4 + p]) for p, v in enumerate(views)]

        return _Phase(2 * NSLAB, pair, edge(0, SHIFT, 0), edge(TAIL0, W - TAIL0, 2),
                      hi_total if _CFG["MERGE"] else None)

    k_phase = functools.partial(kv_phase, k_hbm, kbuf, 0)
    v_phase = functools.partial(kv_phase, v_hbm, vbuf, 1)

    def w_phase(src, dst, bank, ncb, merge):
        cw = src.shape[2] // ncb

        def pair(e, cls):
            nh = _CFG["WHI"]
            s = pl.ds(0, 8 - nh) if cls else pl.ds(8 - nh, nh)
            r = pl.ds(pl.multiple_of((e >> (ncb.bit_length() - 1)) * 8, 8), 8)
            cs = slice(None) if ncb == 1 else pl.ds(pl.multiple_of((e & (ncb - 1)) * cw, 128), cw)
            sm = sem.at[bank, e & (_RING - 1), cls] if cls or not merge else esem.at[bank, 4]
            return copy(src.at[s, r, cs], dst.at[s, r, cs], sm)

        def hi_total():
            v = dst.at[pl.ds(8 - _CFG["WHI"], _CFG["WHI"])]
            return [copy(v, v, esem.at[bank, 4])]

        return _Phase(src.shape[1] // 8 * ncb, pair, hi_total=hi_total if merge else None)

    wm_phase = w_phase(wm_hbm, wm_buf, 0, 4, _CFG["MERGE"])
    wq_phase = w_phase(wq_hbm, wq_buf, 1, 8, _CFG["MERGE"])
    wo_phase = w_phase(wo_hbm, wo_buf, 0, 1, False)

    def loop(n, body):
        def f(i, c):
            body(i)
            return c
        if n == 1:
            body(0)
        elif n > 1:
            lax.fori_loop(0, n, f, 0)

    def run(cur, nxt, compute=None, nbody=0, ppb=0):
        def ahead(t):
            return (cur, t) if t < cur.n else (nxt, t - cur.n)

        def tick(t0, i):
            (p1, t1), (p0, t2) = ahead(t0 + LA1), ahead(t0 + LA0)
            cur.at(t0, i, 1).wait()
            p1.at(t1, i, 1).start(priority=1)
            p0.at(t2, i, 0).start(priority=0)
            if cur.hi_total is None or cur.kind(t0) != "pair":
                cur.at(t0, i, 0).wait()

        def signature(t):
            return [cur.kind(t)] + [(p is cur, p.kind(u)) for p, u in (ahead(t + LA1), ahead(t + LA0))]

        t = 0
        while t < cur.n:
            n = 1
            while t + n < cur.n and signature(t + n) == signature(t):
                n += 1
            if t == cur.first and nbody:
                assert nbody * ppb <= n and t + n + LA1 <= cur.n
                n = nbody * ppb

                def body(i, t=t):
                    for k in range(ppb):
                        tick(t, i * ppb + k)
                        if k == 0:
                            compute(i)
                loop(nbody, body)
            else:
                loop(n, functools.partial(tick, t))
            t += n
        if cur.hi_total is not None:
            for cp in cur.hi_total():
                cp.wait()

    for e in range(LA1):
        wm_phase.pair(e, 1).start(priority=1)
        if e < LA0:
            wm_phase.pair(e, 0).start(priority=0)
    cx = copy(x_hbm, x_buf, fsem.at[0])
    cc = copy(c_hbm, c_buf, fsem.at[1])
    cx.start()
    cc.start()
    run(wm_phase, wq_phase)

    cc.wait()
    cx.wait()
    c = c_buf[...].astype(_F32)
    h_ref[...] = c * jax.nn.sigmoid(c)

    MB, MW = mod_ref.shape[0], mod_ref.shape[2]

    def mod_block(i):
        w = wm_buf[:, :, pl.ds(pl.multiple_of(i * MW, 128), MW)].reshape(D, MW)
        mod_ref[i] = jnp.dot(h_ref[...].astype(_BF16), w, preferred_element_type=_F32)

    run(wq_phase, k_phase(0), mod_block, MB, (wq_phase.n - LA1) // MB)

    def mod(k):
        per = D // MW
        return jnp.concatenate([mod_ref[k * per + t] for t in range(per)], axis=-1)

    h_ref[...] = _layernorm(x_buf[...].astype(_F32)) * (1.0 + mod(1)) + mod(0)

    def q_block(i):
        w = wq_buf[:, :, pl.ds(pl.multiple_of(i * 4 * _DH, 128), 4 * _DH)].reshape(D, 4 * _DH)
        q = jnp.dot(h_ref[...].astype(_BF16), w, preferred_element_type=_F32)
        for t in range(4):
            q_ref[4 * i + t] = q[:, t * _DH:(t + 1) * _DH]

    run(k_phase(0), v_phase(0), q_block, _HQ // 4, PPB)

    def units(g, i):
        if isinstance(i, int):
            gg = (g + (ROT if i == 0 else 0)) & (NG - 1)
        else:
            gg = (g + jnp.where(i == 0, ROT, 0)) & (NG - 1)
        b = gg >> (GPB.bit_length() - 1)
        return [(2 * i + t, b, (gg & (GPB - 1)) * _S + 2 * i + t) for t in range(2)]

    def qk(g, i):
        for u, b, h in units(g, i):
            q = q_ref[h, pl.ds(b, 1), :].astype(_BF16)
            s_ref[pl.ds(u, 1), :] = lax.dot_general(q, kbuf[u], _NT, preferred_element_type=_F32)

    def softmax():
        s = s_ref[...] * scale
        m = jnp.max(s, axis=-1, keepdims=True)
        p = jnp.exp(s - m)
        s_ref[...] = p * (1.0 / jnp.sum(p, axis=-1, keepdims=True))

    def pv(g, i):
        for u, b, h in units(g, i):
            p = s_ref[pl.ds(u, 1), :].astype(_BF16)
            o_ref[h, pl.ds(b, 1), :] = jnp.dot(p, vbuf[u], preferred_element_type=_F32)

    def group(g):
        run(v_phase(g), k_phase(g + 1), functools.partial(qk, g), _S // 2, PPB)
        softmax()
        run(k_phase(g + 1), v_phase(g + 1), functools.partial(pv, g), _S // 2, PPB)

    loop(NG - 1, group)
    run(v_phase(NG - 1), wo_phase, functools.partial(qk, NG - 1), _S // 2, PPB)
    softmax()

    queue = [([wo_phase.pair(e, 1)], wo_phase.pair(e, 0), 4) for e in range(wo_phase.n)]

    FH = F // 2
    NU = FH // _FP
    LAG = _CFG["LAG"]
    blocks = [(r, min(64, FH - r)) for r in range(0, FH, 64)]
    bufs = dict(g=(wg_hbm, wg_buf), u=(wu_hbm, wu_buf), d=(wd_hbm, wd_buf))

    def add(parts):
        si = 2 + 4 * (len(queue) % _FRING)
        cps = []
        for w, half, u in parts:
            rows = pl.ds(u * _FP, _FP)
            idx = slice(None) if half == 2 else half
            cps.append(copy(bufs[w][0].at[idx, rows], bufs[w][1].at[idx, rows], fsem.at[si + len(cps)]))
        queue.append((cps[:-1], cps[-1], sum(2 if half == 2 else 1 for _, half, _ in parts)))

    pos = []
    for i in range(NU + LAG):
        j = i - LAG
        if j < 0:
            add([("g", 2, i), ("u", 0, i), ("u", 1, i)])
        elif i < NU and _CFG["FINE"]:
            add([("g", 2, i), ("u", 1, i)])
            add([("u", 0, i), ("d", 0, j), ("d", 1, j)])
        elif i < NU:
            add([("g", 2, i), ("u", 2, i), ("d", 0, j), ("d", 1, j)])
        else:
            add([("d", 0, j), ("d", 1, j)])
        pos.append(len(queue))
    gu_ready = [pos[(r + n) // _FP - 1] for r, n in blocks]
    d_ready = [pos[(r + n) // _FP - 1 + LAG] for r, n in blocks]
    cum = [0]
    for item in queue:
        cum.append(cum[-1] + item[2])
    waited, started = [0], [LA0, LA1]

    def pump(upto):
        while waited[0] < min(upto, len(queue)):
            e = waited[0]
            for cp in queue[e][0]:
                cp.wait()
            for cls, la in ((1, LA1), (0, LA0)):
                while started[cls] < len(queue) and cum[started[cls]] < cum[e + 1] + 4 * la:
                    assert started[cls] - e < (_RING if started[cls] < wo_phase.n else _FRING)
                    for cp in (queue[started[cls]][0] if cls else [queue[started[cls]][1]]):
                        cp.start(priority=cls)
                    started[cls] += 1
            queue[e][1].wait()
            waited[0] += 1

    for i in range(_S // 2):
        pump(3 * i + 2)
        pv(NG - 1, i)

    attn = jnp.zeros((B, D), _F32)
    for t in range(4):
        pump(max(16 * (t + 1), waited[0] + 4))
        o = jnp.concatenate([o_ref[4 * i + t] for i in range(8)], axis=-1).astype(_BF16)
        w = wo_buf[:, t * _DH:(t + 1) * _DH, :].reshape(8 * _DH, D)
        attn = attn + jnp.dot(o, w, preferred_element_type=_F32)
    pump(waited[0] + 3)

    x1 = x_buf[...].astype(_F32) + mod(2) * attn
    h2 = (_layernorm(x1) * (1.0 + mod(4)) + mod(3)).astype(_BF16)

    def rows_of(buf, r, n):
        return buf[:, r:r + n, :].reshape(2 * n, D)

    hh = []
    y = jnp.zeros((B, D), _F32)
    n_down = 0

    def down(k):
        return jnp.dot(hh[k], rows_of(wd_buf, *blocks[k]), preferred_element_type=_F32)

    for t, (r, n) in enumerate(blocks):
        pump(max(gu_ready[t], waited[0] + 2))
        while n_down < len(hh) and d_ready[n_down] <= waited[0]:
            y = y + down(n_down)
            n_down += 1
        gate = lax.dot_general(h2, rows_of(wg_buf, r, n), _NT, preferred_element_type=_F32)
        up = lax.dot_general(h2, rows_of(wu_buf, r, n), _NT, preferred_element_type=_F32)
        hh.append((jax.nn.sigmoid(gate) * up).astype(_BF16))
    for last in _CFG["CUTS"]:
        last += len(blocks)
        pump(d_ready[last])
        while n_down <= last:
            y = y + down(n_down)
            n_down += 1
    out_ref[...] = (x1 + mod(5) * y).astype(out_ref.dtype)


@jax.jit
def pallas_adaLN_cond__sliding_block_cached__glu_gated_glu__decode_kernel(
    A_x: jax.Array,
    A_k_cache: jax.Array,
    A_v_cache: jax.Array,
    A_wq: jax.Array,
    A_wo: jax.Array,
    B_x: jax.Array,
    B_w_gate: jax.Array,
    B_w_up: jax.Array,
    B_w_down: jax.Array,
    c: jax.Array,
    w_mod: jax.Array,
):
    del B_x
    B, Sq, D = A_x.shape
    Hkv, Sk = A_k_cache.shape[1], A_k_cache.shape[2]
    F = B_w_gate.shape[1]
    assert Sq == 1 and Hkv == _HQ and A_k_cache.shape[3] == _DH
    W = min(4096, max(256, Sk // 4))
    NG = B * _HQ // _S

    x = A_x.reshape(B, D)
    k = A_k_cache.reshape(NG, _S, Sk, _DH)
    v = A_v_cache.reshape(NG, _S, Sk, _DH)
    wq = A_wq.reshape(8, D // 8, _HQ * _DH)
    wo = A_wo.reshape(8, _HQ * _DH // 8, D)
    wm = w_mod.reshape(8, D // 8, 6 * D)
    wg = B_w_gate.T.reshape(2, F // 2, D)
    wu = B_w_up.T.reshape(2, F // 2, D)
    wd = B_w_down.reshape(2, F // 2, D)

    any_spec = pl.BlockSpec(memory_space=pl.ANY)
    out = pl.pallas_call(
        functools.partial(_kernel, B=B, D=D, F=F, Sk=Sk, W=W),
        out_shape=jax.ShapeDtypeStruct(x.shape, x.dtype),
        in_specs=[any_spec] * 10,
        out_specs=pl.BlockSpec(memory_space=pltpu.VMEM),
        scratch_shapes=[
            pltpu.VMEM((_S, W, _DH), _BF16),
            pltpu.VMEM((_S, W, _DH), _BF16),
            pltpu.VMEM(wm.shape, _BF16),
            pltpu.VMEM(wq.shape, _BF16),
            pltpu.VMEM(wo.shape, _BF16),
            pltpu.VMEM(wg.shape, _BF16),
            pltpu.VMEM(wu.shape, _BF16),
            pltpu.VMEM(wd.shape, _BF16),
            pltpu.VMEM(x.shape, _BF16),
            pltpu.VMEM(c.shape, _BF16),
            pltpu.VMEM((12, B, 6 * D // 12), _F32),
            pltpu.VMEM((_HQ, B, _DH), _F32),
            pltpu.VMEM((_HQ, B, _DH), _F32),
            pltpu.VMEM((_S, W), _F32),
            pltpu.VMEM((B, D), _F32),
            pltpu.SemaphoreType.DMA((2, _RING, 2)),
            pltpu.SemaphoreType.DMA((2, 6)),
            pltpu.SemaphoreType.DMA((2 + 4 * _FRING,)),
        ],
        compiler_params=pltpu.CompilerParams(
            vmem_limit_bytes=64 * 1024 * 1024,
            disable_bounds_checks=_CFG.get("FAST", True),
            disable_semaphore_checks=_CFG.get("FAST", True),
        ),
    )(x, k, v, wq, wo, wg, wu, wd, c, wm)
    return out.reshape(A_x.shape)
```

```python
import functools

import jax
import jax.numpy as jnp
from jax import lax
import jax.experimental.pallas as pl
import jax.experimental.pallas.tpu as pltpu

_F32 = jnp.float32
_BF16 = jnp.bfloat16
_NT = (((1,), (1,)), ((), ()))

_HQ = 32
_DH = 128
_EPS = 1e-5
_S = 16
_RING = 32
_FRING = 48
_FP = 16

_CFG = dict(
    R=32,
    SHIFT=8,
    ROT=1,
    LA1=18,
    LA0=9,
    PPB=5,
    SPACE=48,
    HLAG=2,
    LAG=16,
    CUTS=(-3, -1),
)


def _layernorm(x):
    m = jnp.mean(x, axis=-1, keepdims=True)
    xc = x - m
    v = jnp.mean(xc * xc, axis=-1, keepdims=True)
    return xc * lax.rsqrt(v + _EPS)


class _Phase:
    def __init__(self, n, pair, hi_total, head=None, tail=None):
        self.pair, self.hi_total, self.head, self.tail = pair, hi_total, head, tail
        self.first = 0 if head is None else 1
        self.n = n + self.first + (0 if tail is None else 1)

    def kind(self, t):
        if self.head is not None and t == 0:
            return "head"
        if self.tail is not None and t == self.n - 1:
            return "tail"
        return "pair"

    def at(self, t0, i, cls):
        kind = self.kind(t0)
        if kind == "pair":
            return self.pair(t0 - self.first + i, cls)
        return self.head(cls) if kind == "head" else self.tail(cls)


def _kernel(x_hbm, k_hbm, v_hbm, wq_hbm, wo_hbm, wg_hbm, wu_hbm, wd_hbm, c_hbm, wm_hbm,
            out_ref,
            kbuf, vbuf, wm_buf, wq_buf, wo_buf, wg_buf, wu_buf, wd_buf, x_buf, c_buf,
            mod_ref, q_ref, o_ref, s_ref, h_ref, sem, esem, fsem,
            *, B, D, F, Sk, W):
    R, SHIFT, ROT, LA1, LA0, PPB = (_CFG[k] for k in ("R", "SHIFT", "ROT", "LA1", "LA0", "PPB"))
    NG = k_hbm.shape[0]
    GPB = _HQ // _S
    scale = _DH ** -0.5
    copy = pltpu.make_async_copy

    NSLAB = (W - SHIFT) // R
    TAIL0 = SHIFT + NSLAB * R

    def kv_phase(src, dst, bank, g):
        g_of = ((g + ROT) & (NG - 1), g)

        def piece(cls, s, r, n, lo_sem):
            return copy(src.at[g_of[cls], s, pl.ds(Sk - W + r, n), :], dst.at[s, pl.ds(r, n), :],
                        lo_sem if cls else esem.at[bank, 0])

        def pair(e, cls):
            p = e & 1
            return piece(cls, pl.ds(2 + 7 * p, 7) if cls else pl.ds(p, 1),
                         pl.multiple_of(SHIFT + (e >> 1) * R, 8), R, sem.at[bank, e & (_RING - 1)])

        def edge(r, n, k):
            if n == 0:
                return None
            return lambda cls: piece(cls, pl.ds(2, _S - 2) if cls else pl.ds(0, 2), r, n, esem.at[bank, k])

        def hi_total():
            return copy(dst.at[pl.ds(0, 2)], dst.at[pl.ds(0, 2)], esem.at[bank, 0])

        return _Phase(2 * NSLAB, pair, hi_total, edge(0, SHIFT, 1), edge(TAIL0, W - TAIL0, 2))

    k_phase = functools.partial(kv_phase, k_hbm, kbuf, 0)
    v_phase = functools.partial(kv_phase, v_hbm, vbuf, 1)

    def w_phase(src, dst, bank, ncb, hi_sem=None):
        cw = src.shape[2] // ncb

        def pair(e, cls):
            s = pl.ds(0, 7) if cls else pl.ds(7, 1)
            r = pl.ds(pl.multiple_of((e >> (ncb.bit_length() - 1)) * 8, 8), 8)
            cs = slice(None) if ncb == 1 else pl.ds(pl.multiple_of((e & (ncb - 1)) * cw, 128), cw)
            if cls:
                sm = sem.at[bank, e & (_RING - 1)]
            else:
                sm = esem.at[bank, 0] if hi_sem is None else hi_sem(e)
            return copy(src.at[s, r, cs], dst.at[s, r, cs], sm)

        def hi_total():
            return copy(dst.at[pl.ds(7, 1)], dst.at[pl.ds(7, 1)], esem.at[bank, 0])

        return _Phase(src.shape[1] // 8 * ncb, pair, hi_total)

    wm_phase = w_phase(wm_hbm, wm_buf, 0, 4)
    wq_phase = w_phase(wq_hbm, wq_buf, 1, 8)
    wo_phase = w_phase(wo_hbm, wo_buf, 0, 1, lambda e: sem.at[2, e & (_RING - 1)])

    def loop(n, body):
        def f(i, c):
            body(i)
            return c
        if n == 1:
            body(0)
        elif n > 1:
            lax.fori_loop(0, n, f, 0)

    def run(cur, nxt, compute=None, nbody=0, ppb=0):
        def ahead(t):
            return (cur, t) if t < cur.n else (nxt, t - cur.n)

        def tick(t0, i):
            (p1, t1), (p0, t2) = ahead(t0 + LA1), ahead(t0 + LA0)
            cur.at(t0, i, 1).wait()
            p1.at(t1, i, 1).start(priority=1)
            p0.at(t2, i, 0).start(priority=0)

        def signature(t):
            return [cur.kind(t)] + [(p is cur, p.kind(u)) for p, u in (ahead(t + LA1), ahead(t + LA0))]

        t = 0
        while t < cur.n:
            n = 1
            while t + n < cur.n and signature(t + n) == signature(t):
                n += 1
            if t == cur.first and nbody:
                assert nbody * ppb <= n and t + n + LA1 <= cur.n
                n = nbody * ppb

                def body(i, t=t):
                    for k in range(ppb):
                        tick(t, i * ppb + k)
                        if k == 0:
                            compute(i)
                loop(nbody, body)
            else:
                loop(n, functools.partial(tick, t))
            t += n
        cur.hi_total().wait()

    for e in range(LA1):
        wm_phase.pair(e, 1).start(priority=1)
    cx = copy(x_hbm, x_buf, fsem.at[0])
    cc = copy(c_hbm, c_buf, fsem.at[1])
    cx.start()

    def spaced_start(e):
        n = _CFG["SPACE"] * 16
        vbuf[0, pl.ds(0, n), :] = jnp.full((n, _DH), e, jnp.int32).astype(_F32).astype(_BF16)
        wm_phase.pair(e, 0).start(priority=0)

    loop(LA0, spaced_start)
    cc.start()
    run(wm_phase, wq_phase)

    cc.wait()
    cx.wait()
    c = c_buf[...].astype(_F32)
    h_ref[...] = c * jax.nn.sigmoid(c)

    MB, MW = mod_ref.shape[0], mod_ref.shape[2]

    def mod_block(i):
        w = wm_buf[:, :, pl.ds(pl.multiple_of(i * MW, 128), MW)].reshape(D, MW)
        mod_ref[i] = jnp.dot(h_ref[...].astype(_BF16), w, preferred_element_type=_F32)

    run(wq_phase, k_phase(0), mod_block, MB, (wq_phase.n - LA1) // MB)

    def mod(k):
        per = D // MW
        return jnp.concatenate([mod_ref[k * per + t] for t in range(per)], axis=-1)

    h_ref[...] = _layernorm(x_buf[...].astype(_F32)) * (1.0 + mod(1)) + mod(0)

    def q_block(i):
        w = wq_buf[:, :, pl.ds(pl.multiple_of(i * 4 * _DH, 128), 4 * _DH)].reshape(D, 4 * _DH)
        q = jnp.dot(h_ref[...].astype(_BF16), w, preferred_element_type=_F32)
        for t in range(4):
            q_ref[4 * i + t] = q[:, t * _DH:(t + 1) * _DH]

    run(k_phase(0), v_phase(0), q_block, _HQ // 4, PPB)

    def units(g, i):
        if isinstance(i, int):
            gg = (g + (ROT if i == 0 else 0)) & (NG - 1)
        else:
            gg = (g + jnp.where(i == 0, ROT, 0)) & (NG - 1)
        b = gg >> (GPB.bit_length() - 1)
        return [(2 * i + t, b, (gg & (GPB - 1)) * _S + 2 * i + t) for t in range(2)]

    def qk(g, i):
        for u, b, h in units(g, i):
            q = q_ref[h, pl.ds(b, 1), :].astype(_BF16)
            s_ref[pl.ds(u, 1), :] = lax.dot_general(q, kbuf[u], _NT, preferred_element_type=_F32)

    def softmax():
        s = s_ref[...] * scale
        m = jnp.max(s, axis=-1, keepdims=True)
        p = jnp.exp(s - m)
        s_ref[...] = p * (1.0 / jnp.sum(p, axis=-1, keepdims=True))

    def pv(g, i):
        for u, b, h in units(g, i):
            p = s_ref[pl.ds(u, 1), :].astype(_BF16)
            o_ref[h, pl.ds(b, 1), :] = jnp.dot(p, vbuf[u], preferred_element_type=_F32)

    def group(g):
        run(v_phase(g), k_phase(g + 1), functools.partial(qk, g), _S // 2, PPB)
        softmax()
        run(k_phase(g + 1), v_phase(g + 1), functools.partial(pv, g), _S // 2, PPB)

    loop(NG - 1, group)
    run(v_phase(NG - 1), wo_phase, functools.partial(qk, NG - 1), _S // 2, PPB)
    softmax()

    queue = [([wo_phase.pair(e, 1)], wo_phase.pair(e, 0), 4) for e in range(wo_phase.n)]

    FH = F // 2
    NU = FH // _FP
    LAG = _CFG["LAG"]
    blocks = [(r, min(64, FH - r)) for r in range(0, FH, 64)]
    bufs = dict(g=(wg_hbm, wg_buf), u=(wu_hbm, wu_buf), d=(wd_hbm, wd_buf))

    def add(parts):
        si = 2 + 4 * (len(queue) % _FRING)
        cps = []
        for w, half, u in parts:
            rows = pl.ds(u * _FP, _FP)
            idx = slice(None) if half == 2 else half
            cps.append(copy(bufs[w][0].at[idx, rows], bufs[w][1].at[idx, rows], fsem.at[si + len(cps)]))
        queue.append((cps[:-1], cps[-1], sum(2 if half == 2 else 1 for _, half, _ in parts)))

    pos = []
    for i in range(NU + LAG):
        j = i - LAG
        if j < 0:
            add([("g", 2, i), ("u", 0, i), ("u", 1, i)])
        elif i < NU:
            add([("g", 2, i), ("u", 2, i), ("d", 0, j), ("d", 1, j)])
        else:
            add([("d", 0, j), ("d", 1, j)])
        pos.append(len(queue))
    gu_ready = [pos[(r + n) // _FP - 1] for r, n in blocks]
    d_ready = [pos[(r + n) // _FP - 1 + LAG] for r, n in blocks]
    cum = [0]
    for item in queue:
        cum.append(cum[-1] + item[2])
    waited, started = [0, 0], [LA0, LA1]
    ELA0 = _CFG.get("ELA0", LA0)

    def pump(upto, need=0):
        while waited[1] < min(max(upto, need), len(queue)):
            e = waited[1]
            while waited[0] < (need if e == need - 1 else e - _CFG["HLAG"]):
                queue[waited[0]][1].wait()
                waited[0] += 1
            for cp in queue[e][0]:
                cp.wait()
            waited[1] += 1
            for cls, la in ((1, LA1), (0, ELA0)):
                while started[cls] < len(queue) and cum[started[cls]] < cum[e + 1] + 4 * la:
                    ring = _RING if started[cls] < wo_phase.n else _FRING
                    assert started[cls] - waited[cls] < ring
                    for cp in (queue[started[cls]][0] if cls else [queue[started[cls]][1]]):
                        cp.start(priority=cls)
                    started[cls] += 1
        while waited[0] < need:
            queue[waited[0]][1].wait()
            waited[0] += 1

    for i in range(_S // 2):
        pump(3 * i + 2)
        pv(NG - 1, i)

    attn = jnp.zeros((B, D), _F32)
    for t in range(4):
        pump(waited[1] + 4, 16 * (t + 1))
        o = jnp.concatenate([o_ref[4 * i + t] for i in range(8)], axis=-1).astype(_BF16)
        w = wo_buf[:, t * _DH:(t + 1) * _DH, :].reshape(8 * _DH, D)
        attn = attn + jnp.dot(o, w, preferred_element_type=_F32)
    pump(waited[1] + 3)

    x1 = x_buf[...].astype(_F32) + mod(2) * attn
    h2 = (_layernorm(x1) * (1.0 + mod(4)) + mod(3)).astype(_BF16)

    def rows_of(buf, r, n):
        return buf[:, r:r + n, :].reshape(2 * n, D)

    hh = []
    y = jnp.zeros((B, D), _F32)
    n_down = 0

    def down(k):
        return jnp.dot(hh[k], rows_of(wd_buf, *blocks[k]), preferred_element_type=_F32)

    for t, (r, n) in enumerate(blocks):
        pump(waited[1] + 2, gu_ready[t])
        while n_down < len(hh) and d_ready[n_down] <= waited[0]:
            y = y + down(n_down)
            n_down += 1
        gate = lax.dot_general(h2, rows_of(wg_buf, r, n), _NT, preferred_element_type=_F32)
        up = lax.dot_general(h2, rows_of(wu_buf, r, n), _NT, preferred_element_type=_F32)
        hh.append((jax.nn.sigmoid(gate) * up).astype(_BF16))
    for last in _CFG["CUTS"]:
        last += len(blocks)
        pump(0, d_ready[last])
        while n_down <= last:
            y = y + down(n_down)
            n_down += 1
    out_ref[...] = (x1 + mod(5) * y).astype(out_ref.dtype)


@jax.jit
def pallas_adaLN_cond__sliding_block_cached__glu_gated_glu__decode_kernel(
    A_x: jax.Array,
    A_k_cache: jax.Array,
    A_v_cache: jax.Array,
    A_wq: jax.Array,
    A_wo: jax.Array,
    B_x: jax.Array,
    B_w_gate: jax.Array,
    B_w_up: jax.Array,
    B_w_down: jax.Array,
    c: jax.Array,
    w_mod: jax.Array,
):
    del B_x
    B, Sq, D = A_x.shape
    Hkv, Sk = A_k_cache.shape[1], A_k_cache.shape[2]
    F = B_w_gate.shape[1]
    assert Sq == 1 and Hkv == _HQ and A_k_cache.shape[3] == _DH
    W = min(4096, max(256, Sk // 4))
    NG = B * _HQ // _S

    x = A_x.reshape(B, D)
    k = A_k_cache.reshape(NG, _S, Sk, _DH)
    v = A_v_cache.reshape(NG, _S, Sk, _DH)
    wq = A_wq.reshape(8, D // 8, _HQ * _DH)
    wo = A_wo.reshape(8, _HQ * _DH // 8, D)
    wm = w_mod.reshape(8, D // 8, 6 * D)
    wg = B_w_gate.T.reshape(2, F // 2, D)
    wu = B_w_up.T.reshape(2, F // 2, D)
    wd = B_w_down.reshape(2, F // 2, D)

    any_spec = pl.BlockSpec(memory_space=pl.ANY)
    out = pl.pallas_call(
        functools.partial(_kernel, B=B, D=D, F=F, Sk=Sk, W=W),
        out_shape=jax.ShapeDtypeStruct(x.shape, x.dtype),
        in_specs=[any_spec] * 10,
        out_specs=pl.BlockSpec(memory_space=pltpu.VMEM),
        scratch_shapes=[
            pltpu.VMEM((_S, W, _DH), _BF16),
            pltpu.VMEM((_S, W, _DH), _BF16),
            pltpu.VMEM(wm.shape, _BF16),
            pltpu.VMEM(wq.shape, _BF16),
            pltpu.VMEM(wo.shape, _BF16),
            pltpu.VMEM(wg.shape, _BF16),
            pltpu.VMEM(wu.shape, _BF16),
            pltpu.VMEM(wd.shape, _BF16),
            pltpu.VMEM(x.shape, _BF16),
            pltpu.VMEM(c.shape, _BF16),
            pltpu.VMEM((12, B, 6 * D // 12), _F32),
            pltpu.VMEM((_HQ, B, _DH), _F32),
            pltpu.VMEM((_HQ, B, _DH), _F32),
            pltpu.VMEM((_S, W), _F32),
            pltpu.VMEM((B, D), _F32),
            pltpu.SemaphoreType.DMA((3, _RING)),
            pltpu.SemaphoreType.DMA((2, 3)),
            pltpu.SemaphoreType.DMA((2 + 4 * _FRING,)),
        ],
        compiler_params=pltpu.CompilerParams(
            vmem_limit_bytes=64 * 1024 * 1024,
            disable_bounds_checks=_CFG.get("FAST", True),
            disable_semaphore_checks=_CFG.get("FAST", True),
        ),
    )(x, k, v, wq, wo, wg, wu, wd, c, wm)
    return out.reshape(A_x.shape)
```

```python
import functools

import jax
import jax.numpy as jnp
from jax import lax
import jax.experimental.pallas as pl
import jax.experimental.pallas.tpu as pltpu

_F32 = jnp.float32
_BF16 = jnp.bfloat16
_NT = (((1,), (1,)), ((), ()))

_HQ = 32
_DH = 128
_EPS = 1e-5
_S = 16
_RING = 32
_FP = 16

_CFG = dict(
    R=32,
    SHIFT=8,
    ROT=1,
    LA1=18,
    LA0=9,
    PPB=5,
    SPACE=48,
    HLAG=2,
    LAG=16,
    CUTS=(-3, -1),
    CHECKS=False,
)


def _layernorm(x):
    m = jnp.mean(x, axis=-1, keepdims=True)
    xc = x - m
    v = jnp.mean(xc * xc, axis=-1, keepdims=True)
    return xc * lax.rsqrt(v + _EPS)


class _Phase:
    def __init__(self, n, pair, hi_total, head=None, tail=None):
        self.pair, self.hi_total, self.head, self.tail = pair, hi_total, head, tail
        self.first = 0 if head is None else 1
        self.n = n + self.first + (0 if tail is None else 1)

    def kind(self, t):
        if self.head is not None and t == 0:
            return "head"
        if self.tail is not None and t == self.n - 1:
            return "tail"
        return "pair"

    def at(self, t0, i, cls):
        kind = self.kind(t0)
        if kind == "pair":
            return self.pair(t0 - self.first + i, cls)
        return self.head(cls) if kind == "head" else self.tail(cls)


def _kernel(x_hbm, k_hbm, v_hbm, wq_hbm, wo_hbm, wg_hbm, wu_hbm, wd_hbm, c_hbm, wm_hbm,
            out_ref,
            kbuf, vbuf, wm_buf, wq_buf, wo_buf, wg_buf, wu_buf, wd_buf, x_buf, c_buf,
            mod_ref, q_ref, o_ref, s_ref, h_ref, sem, esem, fsem,
            *, B, D, F, Sk, W):
    R, SHIFT, ROT, LA1, LA0, PPB = (_CFG[k] for k in ("R", "SHIFT", "ROT", "LA1", "LA0", "PPB"))
    NG = k_hbm.shape[0]
    GPB = _HQ // _S
    scale = _DH ** -0.5
    copy = pltpu.make_async_copy

    NSLAB = (W - SHIFT) // R
    TAIL0 = SHIFT + NSLAB * R

    def kv_phase(src, dst, bank, g):
        g_of = ((g + ROT) & (NG - 1), g)

        def piece(cls, s, r, n, lo_sem):
            return copy(src.at[g_of[cls], s, pl.ds(Sk - W + r, n), :], dst.at[s, pl.ds(r, n), :],
                        lo_sem if cls else esem.at[bank, 0])

        def pair(e, cls):
            p = e & 1
            return piece(cls, pl.ds(2 + 7 * p, 7) if cls else pl.ds(p, 1),
                         pl.multiple_of(SHIFT + (e >> 1) * R, 8), R, sem.at[bank, e & (_RING - 1)])

        def edge(r, n, k):
            if n == 0:
                return None
            return lambda cls: piece(cls, pl.ds(2, _S - 2) if cls else pl.ds(0, 2), r, n, esem.at[bank, k])

        def hi_total():
            return copy(dst.at[pl.ds(0, 2)], dst.at[pl.ds(0, 2)], esem.at[bank, 0])

        return _Phase(2 * NSLAB, pair, hi_total, edge(0, SHIFT, 1), edge(TAIL0, W - TAIL0, 2))

    k_phase = functools.partial(kv_phase, k_hbm, kbuf, 0)
    v_phase = functools.partial(kv_phase, v_hbm, vbuf, 1)

    def w_phase(src, dst, bank, ncb, hi_sem=None):
        cw = src.shape[2] // ncb

        def pair(e, cls):
            s = pl.ds(0, 7) if cls else pl.ds(7, 1)
            r = pl.ds(pl.multiple_of((e >> (ncb.bit_length() - 1)) * 8, 8), 8)
            cs = slice(None) if ncb == 1 else pl.ds(pl.multiple_of((e & (ncb - 1)) * cw, 128), cw)
            if cls:
                sm = sem.at[bank, e & (_RING - 1)]
            else:
                sm = esem.at[bank, 0] if hi_sem is None else hi_sem(e)
            return copy(src.at[s, r, cs], dst.at[s, r, cs], sm)

        def hi_total():
            return copy(dst.at[pl.ds(7, 1)], dst.at[pl.ds(7, 1)], esem.at[bank, 0])

        return _Phase(src.shape[1] // 8 * ncb, pair, hi_total)

    wm_phase = w_phase(wm_hbm, wm_buf, 0, 4)
    wq_phase = w_phase(wq_hbm, wq_buf, 1, 8)
    wo_phase = w_phase(wo_hbm, wo_buf, 0, 1, lambda e: sem.at[2, e & (_RING - 1)])

    def loop(n, body):
        def f(i, c):
            body(i)
            return c
        if n == 1:
            body(0)
        elif n > 1:
            lax.fori_loop(0, n, f, 0)

    def run(cur, nxt, compute=None, nbody=0, ppb=0):
        def ahead(t):
            return (cur, t) if t < cur.n else (nxt, t - cur.n)

        def tick(t0, i):
            (p1, t1), (p0, t2) = ahead(t0 + LA1), ahead(t0 + LA0)
            cur.at(t0, i, 1).wait()
            p1.at(t1, i, 1).start(priority=1)
            p0.at(t2, i, 0).start(priority=0)

        def signature(t):
            return [cur.kind(t)] + [(p is cur, p.kind(u)) for p, u in (ahead(t + LA1), ahead(t + LA0))]

        t = 0
        while t < cur.n:
            n = 1
            while t + n < cur.n and signature(t + n) == signature(t):
                n += 1
            if t == cur.first and nbody:
                assert nbody * ppb <= n and t + n + LA1 <= cur.n
                n = nbody * ppb

                def body(i, t=t):
                    for k in range(ppb):
                        tick(t, i * ppb + k)
                        if k == 0:
                            compute(i)
                loop(nbody, body)
            else:
                loop(n, functools.partial(tick, t))
            t += n
        cur.hi_total().wait()

    for e in range(LA1):
        wm_phase.pair(e, 1).start(priority=1)
    cx = copy(x_hbm, x_buf, fsem.at[0])
    cc = copy(c_hbm, c_buf, fsem.at[1])
    cx.start()

    def spaced_start(e):
        n = _CFG["SPACE"] * 16
        vbuf[0, pl.ds(0, n), :] = jnp.full((n, _DH), e, jnp.int32).astype(_F32).astype(_BF16)
        wm_phase.pair(e, 0).start(priority=0)

    loop(LA0, spaced_start)
    cc.start()
    run(wm_phase, wq_phase)

    cc.wait()
    cx.wait()
    c = c_buf[...].astype(_F32)
    h_ref[...] = c * jax.nn.sigmoid(c)

    MB, MW = mod_ref.shape[0], mod_ref.shape[2]

    def mod_block(i):
        w = wm_buf[:, :, pl.ds(pl.multiple_of(i * MW, 128), MW)].reshape(D, MW)
        mod_ref[i] = jnp.dot(h_ref[...].astype(_BF16), w, preferred_element_type=_F32)

    run(wq_phase, k_phase(0), mod_block, MB, (wq_phase.n - LA1) // MB)

    def mod(k):
        per = D // MW
        return jnp.concatenate([mod_ref[k * per + t] for t in range(per)], axis=-1)

    h_ref[...] = _layernorm(x_buf[...].astype(_F32)) * (1.0 + mod(1)) + mod(0)

    def q_block(i):
        w = wq_buf[:, :, pl.ds(pl.multiple_of(i * 4 * _DH, 128), 4 * _DH)].reshape(D, 4 * _DH)
        q = jnp.dot(h_ref[...].astype(_BF16), w, preferred_element_type=_F32)
        for t in range(4):
            q_ref[4 * i + t] = q[:, t * _DH:(t + 1) * _DH]

    run(k_phase(0), v_phase(0), q_block, _HQ // 4, PPB)

    def units(g, i):
        if isinstance(i, int):
            gg = (g + (ROT if i == 0 else 0)) & (NG - 1)
        else:
            gg = (g + jnp.where(i == 0, ROT, 0)) & (NG - 1)
        b = gg >> (GPB.bit_length() - 1)
        return [(2 * i + t, b, (gg & (GPB - 1)) * _S + 2 * i + t) for t in range(2)]

    def qk(g, i):
        for u, b, h in units(g, i):
            q = q_ref[h, pl.ds(b, 1), :].astype(_BF16)
            s_ref[pl.ds(u, 1), :] = lax.dot_general(q, kbuf[u], _NT, preferred_element_type=_F32)

    def softmax():
        s = s_ref[...] * scale
        m = jnp.max(s, axis=-1, keepdims=True)
        p = jnp.exp(s - m)
        s_ref[...] = p * (1.0 / jnp.sum(p, axis=-1, keepdims=True))

    def pv(g, i):
        for u, b, h in units(g, i):
            p = s_ref[pl.ds(u, 1), :].astype(_BF16)
            o_ref[h, pl.ds(b, 1), :] = jnp.dot(p, vbuf[u], preferred_element_type=_F32)

    def group(g):
        run(v_phase(g), k_phase(g + 1), functools.partial(qk, g), _S // 2, PPB)
        softmax()
        run(k_phase(g + 1), v_phase(g + 1), functools.partial(pv, g), _S // 2, PPB)

    loop(NG - 1, group)
    run(v_phase(NG - 1), wo_phase, functools.partial(qk, NG - 1), _S // 2, PPB)
    softmax()

    queue = [([wo_phase.pair(e, 1)], wo_phase.pair(e, 0), 4) for e in range(wo_phase.n)]

    FH = F // 2
    NU = FH // _FP
    LAG = _CFG["LAG"]
    blocks = [(r, min(64, FH - r)) for r in range(0, FH, 64)]
    bufs = dict(g=(wg_hbm, wg_buf), u=(wu_hbm, wu_buf), d=(wd_hbm, wd_buf))

    def add(parts):
        si = 2 + 4 * (len(queue) - wo_phase.n)
        cps = []
        for w, half, u in parts:
            rows = pl.ds(u * _FP, _FP)
            idx = slice(None) if half == 2 else half
            cps.append(copy(bufs[w][0].at[idx, rows], bufs[w][1].at[idx, rows], fsem.at[si + len(cps)]))
        queue.append((cps[:-1], cps[-1], sum(2 if half == 2 else 1 for _, half, _ in parts)))

    pos = []
    for i in range(NU + LAG):
        j = i - LAG
        if j < 0:
            add([("g", 2, i), ("u", 0, i), ("u", 1, i)])
        elif i < NU:
            add([("g", 2, i), ("u", 2, i), ("d", 0, j), ("d", 1, j)])
        else:
            add([("d", 0, j), ("d", 1, j)])
        pos.append(len(queue))
    gu_ready = [pos[(r + n) // _FP - 1] for r, n in blocks]
    d_ready = [pos[(r + n) // _FP - 1 + LAG] for r, n in blocks]
    cum = [0]
    for item in queue:
        cum.append(cum[-1] + item[2])
    waited, started = [0, 0], [LA0, LA1]

    def pump(upto, need=0):
        while waited[1] < min(max(upto, need), len(queue)):
            e = waited[1]
            while waited[0] < (need if e == need - 1 else e - _CFG["HLAG"]):
                queue[waited[0]][1].wait()
                waited[0] += 1
            for cp in queue[e][0]:
                cp.wait()
            waited[1] += 1
            for cls, la in ((1, LA1), (0, LA0)):
                while started[cls] < len(queue) and cum[started[cls]] < cum[e + 1] + 4 * la:
                    assert started[cls] >= wo_phase.n or started[cls] - waited[cls] < _RING
                    for cp in (queue[started[cls]][0] if cls else [queue[started[cls]][1]]):
                        cp.start(priority=cls)
                    started[cls] += 1
        while waited[0] < need:
            queue[waited[0]][1].wait()
            waited[0] += 1

    for i in range(_S // 2):
        pump(3 * i + 2)
        pv(NG - 1, i)

    attn = jnp.zeros((B, D), _F32)
    for t in range(4):
        pump(waited[1] + 4, 16 * (t + 1))
        o = jnp.concatenate([o_ref[4 * i + t] for i in range(8)], axis=-1).astype(_BF16)
        w = wo_buf[:, t * _DH:(t + 1) * _DH, :].reshape(8 * _DH, D)
        attn = attn + jnp.dot(o, w, preferred_element_type=_F32)
    pump(waited[1] + 3)

    x1 = x_buf[...].astype(_F32) + mod(2) * attn
    h2 = (_layernorm(x1) * (1.0 + mod(4)) + mod(3)).astype(_BF16)

    def rows_of(buf, r, n):
        return buf[:, r:r + n, :].reshape(2 * n, D)

    hh = []
    y = jnp.zeros((B, D), _F32)
    n_down = 0

    def down(k):
        return jnp.dot(hh[k], rows_of(wd_buf, *blocks[k]), preferred_element_type=_F32)

    for t, (r, n) in enumerate(blocks):
        pump(waited[1] + 2, gu_ready[t])
        while n_down < len(hh) and d_ready[n_down] <= waited[0]:
            y = y + down(n_down)
            n_down += 1
        gate = lax.dot_general(h2, rows_of(wg_buf, r, n), _NT, preferred_element_type=_F32)
        up = lax.dot_general(h2, rows_of(wu_buf, r, n), _NT, preferred_element_type=_F32)
        hh.append((jax.nn.sigmoid(gate) * up).astype(_BF16))
    for last in _CFG["CUTS"]:
        last += len(blocks)
        pump(0, d_ready[last])
        while n_down <= last:
            y = y + down(n_down)
            n_down += 1
    assert waited == [len(queue)] * 2 and n_down == len(blocks)
    out_ref[...] = (x1 + mod(5) * y).astype(out_ref.dtype)


@jax.jit
def pallas_adaLN_cond__sliding_block_cached__glu_gated_glu__decode_kernel(
    A_x: jax.Array,
    A_k_cache: jax.Array,
    A_v_cache: jax.Array,
    A_wq: jax.Array,
    A_wo: jax.Array,
    B_x: jax.Array,
    B_w_gate: jax.Array,
    B_w_up: jax.Array,
    B_w_down: jax.Array,
    c: jax.Array,
    w_mod: jax.Array,
):
    del B_x
    B, Sq, D = A_x.shape
    Hkv, Sk = A_k_cache.shape[1], A_k_cache.shape[2]
    F = B_w_gate.shape[1]
    assert Sq == 1 and Hkv == _HQ and A_k_cache.shape[3] == _DH
    assert (B, D, Sk) == (8, 512, 4096) and F % (2 * _FP) == 0
    W = min(4096, max(256, Sk // 4))
    NG = B * _HQ // _S

    x = A_x.reshape(B, D)
    k = A_k_cache.reshape(NG, _S, Sk, _DH)
    v = A_v_cache.reshape(NG, _S, Sk, _DH)
    wq = A_wq.reshape(8, D // 8, _HQ * _DH)
    wo = A_wo.reshape(8, _HQ * _DH // 8, D)
    wm = w_mod.reshape(8, D // 8, 6 * D)
    wg = B_w_gate.T.reshape(2, F // 2, D)
    wu = B_w_up.T.reshape(2, F // 2, D)
    wd = B_w_down.reshape(2, F // 2, D)

    any_spec = pl.BlockSpec(memory_space=pl.ANY)
    out = pl.pallas_call(
        functools.partial(_kernel, B=B, D=D, F=F, Sk=Sk, W=W),
        out_shape=jax.ShapeDtypeStruct(x.shape, x.dtype),
        in_specs=[any_spec] * 10,
        out_specs=pl.BlockSpec(memory_space=pltpu.VMEM),
        scratch_shapes=[
            pltpu.VMEM((_S, W, _DH), _BF16),
            pltpu.VMEM((_S, W, _DH), _BF16),
            pltpu.VMEM(wm.shape, _BF16),
            pltpu.VMEM(wq.shape, _BF16),
            pltpu.VMEM(wo.shape, _BF16),
            pltpu.VMEM(wg.shape, _BF16),
            pltpu.VMEM(wu.shape, _BF16),
            pltpu.VMEM(wd.shape, _BF16),
            pltpu.VMEM(x.shape, _BF16),
            pltpu.VMEM(c.shape, _BF16),
            pltpu.VMEM((12, B, 6 * D // 12), _F32),
            pltpu.VMEM((_HQ, B, _DH), _F32),
            pltpu.VMEM((_HQ, B, _DH), _F32),
            pltpu.VMEM((_S, W), _F32),
            pltpu.VMEM((B, D), _F32),
            pltpu.SemaphoreType.DMA((3, _RING)),
            pltpu.SemaphoreType.DMA((2, 3)),
            pltpu.SemaphoreType.DMA((2 + 4 * (F // 2 // _FP + _CFG["LAG"]),)),
        ],
        compiler_params=pltpu.CompilerParams(
            vmem_limit_bytes=64 * 1024 * 1024,
            disable_bounds_checks=not _CFG["CHECKS"],
            disable_semaphore_checks=not _CFG["CHECKS"],
        ),
    )(x, k, v, wq, wo, wg, wu, wd, c, wm)
    return out.reshape(A_x.shape)
```

```python
import functools

import jax
import jax.numpy as jnp
from jax import lax
import jax.experimental.pallas as pl
import jax.experimental.pallas.tpu as pltpu

_F32 = jnp.float32
_BF16 = jnp.bfloat16
_NT = (((1,), (1,)), ((), ()))

_HQ = 32
_DH = 128
_EPS = 1e-5
_S = 16
_RING = 32
_FP = 16

_CFG = dict(
    R=32,
    SHIFT=8,
    ROT=1,
    LA1=18,
    LA0=9,
    PPB=5,
    SPACE=48,
    HLAG=2,
    LAG=16,
    CUTS=(-3, -1),
    CHECKS=False,
)


def _layernorm(x):
    m = jnp.mean(x, axis=-1, keepdims=True)
    xc = x - m
    v = jnp.mean(xc * xc, axis=-1, keepdims=True)
    return xc * lax.rsqrt(v + _EPS)


class _Phase:
    def __init__(self, n, pair, hi_total, head=None, tail=None):
        self.pair, self.hi_total, self.head, self.tail = pair, hi_total, head, tail
        self.first = 0 if head is None else 1
        self.n = n + self.first + (0 if tail is None else 1)

    def kind(self, t):
        if self.head is not None and t == 0:
            return "head"
        if self.tail is not None and t == self.n - 1:
            return "tail"
        return "pair"

    def at(self, t0, i, cls):
        kind = self.kind(t0)
        if kind == "pair":
            return self.pair(t0 - self.first + i, cls)
        return self.head(cls) if kind == "head" else self.tail(cls)


def _kernel(x_hbm, k_hbm, v_hbm, wq_hbm, wo_hbm, wg_hbm, wu_hbm, wd_hbm, c_hbm, wm_hbm,
            out_ref,
            kbuf, vbuf, wm_buf, wq_buf, wo_buf, wg_buf, wu_buf, wd_buf, x_buf, c_buf,
            mod_ref, q_ref, o_ref, s_ref, h_ref, sem, esem, fsem,
            *, B, D, F, Sk, W):
    R, SHIFT, ROT, LA1, LA0, PPB = (_CFG[k] for k in ("R", "SHIFT", "ROT", "LA1", "LA0", "PPB"))
    NG = k_hbm.shape[0]
    GPB = _HQ // _S
    scale = _DH ** -0.5
    copy = pltpu.make_async_copy

    NSLAB = (W - SHIFT) // R
    TAIL0 = SHIFT + NSLAB * R

    def kv_phase(src, dst, bank, g):
        g_of = ((g + ROT) & (NG - 1), g)

        def piece(cls, s, r, n, lo_sem):
            return copy(src.at[g_of[cls], s, pl.ds(Sk - W + r, n), :], dst.at[s, pl.ds(r, n), :],
                        lo_sem if cls else esem.at[bank, 0])

        def pair(e, cls):
            p = e & 1
            return piece(cls, pl.ds(2 + 7 * p, 7) if cls else pl.ds(p, 1),
                         pl.multiple_of(SHIFT + (e >> 1) * R, 8), R, sem.at[bank, e & (_RING - 1)])

        def edge(r, n, k):
            if n == 0:
                return None
            return lambda cls: piece(cls, pl.ds(2, _S - 2) if cls else pl.ds(0, 2), r, n, esem.at[bank, k])

        def hi_total():
            return copy(dst.at[pl.ds(0, 2)], dst.at[pl.ds(0, 2)], esem.at[bank, 0])

        return _Phase(2 * NSLAB, pair, hi_total, edge(0, SHIFT, 1), edge(TAIL0, W - TAIL0, 2))

    k_phase = functools.partial(kv_phase, k_hbm, kbuf, 0)
    v_phase = functools.partial(kv_phase, v_hbm, vbuf, 1)

    def w_phase(src, dst, bank, ncb, hi_sem=None):
        cw = src.shape[2] // ncb

        def pair(e, cls):
            s = pl.ds(0, 7) if cls else pl.ds(7, 1)
            r = pl.ds(pl.multiple_of((e >> (ncb.bit_length() - 1)) * 8, 8), 8)
            cs = slice(None) if ncb == 1 else pl.ds(pl.multiple_of((e & (ncb - 1)) * cw, 128), cw)
            if cls:
                sm = sem.at[bank, e & (_RING - 1)]
            else:
                sm = esem.at[bank, 0] if hi_sem is None else hi_sem(e)
            return copy(src.at[s, r, cs], dst.at[s, r, cs], sm)

        def hi_total():
            return copy(dst.at[pl.ds(7, 1)], dst.at[pl.ds(7, 1)], esem.at[bank, 0])

        return _Phase(src.shape[1] // 8 * ncb, pair, hi_total)

    wm_phase = w_phase(wm_hbm, wm_buf, 0, 4)
    wq_phase = w_phase(wq_hbm, wq_buf, 1, 8)
    wo_phase = w_phase(wo_hbm, wo_buf, 0, 1, lambda e: sem.at[2, e & (_RING - 1)])

    def loop(n, body):
        def f(i, c):
            body(i)
            return c
        if n == 1:
            body(0)
        elif n > 1:
            lax.fori_loop(0, n, f, 0)

    def run(cur, nxt, compute=None, nbody=0, ppb=0, after=None):
        def ahead(t):
            return (cur, t) if t < cur.n else (nxt, t - cur.n)

        def tick(t0, i):
            (p1, t1), (p0, t2) = ahead(t0 + LA1), ahead(t0 + LA0)
            cur.at(t0, i, 1).wait()
            p1.at(t1, i, 1).start(priority=1)
            p0.at(t2, i, 0).start(priority=0)

        def signature(t):
            return [cur.kind(t)] + [(p is cur, p.kind(u)) for p, u in (ahead(t + LA1), ahead(t + LA0))]

        t = 0
        while t < cur.n:
            n = 1
            while t + n < cur.n and signature(t + n) == signature(t):
                n += 1
            if t == cur.first and nbody:
                assert nbody * ppb <= n and t + n + LA1 <= cur.n
                n = nbody * ppb

                def body(i, t=t):
                    for k in range(ppb):
                        tick(t, i * ppb + k)
                        if k == 0:
                            compute(i)
                loop(nbody, body)
                if after is not None:
                    after()
            else:
                loop(n, functools.partial(tick, t))
            t += n
        cur.hi_total().wait()

    for e in range(LA1):
        wm_phase.pair(e, 1).start(priority=1)
    cx = copy(x_hbm, x_buf, fsem.at[0])
    cc = copy(c_hbm, c_buf, fsem.at[1])
    cx.start()

    def spaced_start(e):
        n = _CFG["SPACE"] * 16
        vbuf[0, pl.ds(0, n), :] = jnp.full((n, _DH), e, jnp.int32).astype(_F32).astype(_BF16)
        wm_phase.pair(e, 0).start(priority=0)

    loop(LA0, spaced_start)
    cc.start()
    run(wm_phase, wq_phase)

    cc.wait()
    cx.wait()
    c = c_buf[...].astype(_F32)
    h_ref[...] = c * jax.nn.sigmoid(c)

    MB, MW = mod_ref.shape[0], mod_ref.shape[2]

    def mod_block(i):
        w = wm_buf[:, :, pl.ds(pl.multiple_of(i * MW, 128), MW)].reshape(D, MW)
        mod_ref[i] = jnp.dot(h_ref[...].astype(_BF16), w, preferred_element_type=_F32)

    run(wq_phase, k_phase(0), mod_block, MB, (wq_phase.n - LA1) // MB)

    def mod(k):
        per = D // MW
        return jnp.concatenate([mod_ref[k * per + t] for t in range(per)], axis=-1)

    h_ref[...] = _layernorm(x_buf[...].astype(_F32)) * (1.0 + mod(1)) + mod(0)

    def q_block(i):
        w = wq_buf[:, :, pl.ds(pl.multiple_of(i * 4 * _DH, 128), 4 * _DH)].reshape(D, 4 * _DH)
        q = jnp.dot(h_ref[...].astype(_BF16), w, preferred_element_type=_F32)
        for t in range(4):
            q_ref[4 * i + t] = q[:, t * _DH:(t + 1) * _DH]

    run(k_phase(0), v_phase(0), q_block, _HQ // 4, PPB)

    def units(g, i):
        if isinstance(i, int):
            gg = (g + (ROT if i == 0 else 0)) & (NG - 1)
        else:
            gg = (g + jnp.where(i == 0, ROT, 0)) & (NG - 1)
        b = gg >> (GPB.bit_length() - 1)
        return [(2 * i + t, b, (gg & (GPB - 1)) * _S + 2 * i + t) for t in range(2)]

    def qk(g, i):
        for u, b, h in units(g, i):
            q = q_ref[h, pl.ds(b, 1), :].astype(_BF16)
            s_ref[pl.ds(u, 1), :] = lax.dot_general(q, kbuf[u], _NT, preferred_element_type=_F32)

    def softmax():
        s = s_ref[...] * scale
        m = jnp.max(s, axis=-1, keepdims=True)
        p = jnp.exp(s - m)
        s_ref[...] = p * (1.0 / jnp.sum(p, axis=-1, keepdims=True))

    def pv(g, i):
        for u, b, h in units(g, i):
            p = s_ref[pl.ds(u, 1), :].astype(_BF16)
            o_ref[h, pl.ds(b, 1), :] = jnp.dot(p, vbuf[u], preferred_element_type=_F32)

    def group(g):
        run(v_phase(g), k_phase(g + 1), functools.partial(qk, g), _S // 2, PPB, softmax)
        run(k_phase(g + 1), v_phase(g + 1), functools.partial(pv, g), _S // 2, PPB)

    loop(NG - 1, group)
    run(v_phase(NG - 1), wo_phase, functools.partial(qk, NG - 1), _S // 2, PPB, softmax)

    queue = [([wo_phase.pair(e, 1)], wo_phase.pair(e, 0), 4) for e in range(wo_phase.n)]

    FH = F // 2
    NU = FH // _FP
    LAG = _CFG["LAG"]
    blocks = [(r, min(64, FH - r)) for r in range(0, FH, 64)]
    bufs = dict(g=(wg_hbm, wg_buf), u=(wu_hbm, wu_buf), d=(wd_hbm, wd_buf))

    def add(parts):
        si = 2 + 4 * (len(queue) - wo_phase.n)
        cps = []
        for w, half, u in parts:
            rows = pl.ds(u * _FP, _FP)
            idx = slice(None) if half == 2 else half
            cps.append(copy(bufs[w][0].at[idx, rows], bufs[w][1].at[idx, rows], fsem.at[si + len(cps)]))
        queue.append((cps[:-1], cps[-1], sum(2 if half == 2 else 1 for _, half, _ in parts)))

    pos = []
    for i in range(NU + LAG):
        j = i - LAG
        if j < 0:
            add([("g", 2, i), ("u", 0, i), ("u", 1, i)])
        elif i < NU:
            add([("g", 2, i), ("u", 2, i), ("d", 0, j), ("d", 1, j)])
        else:
            add([("d", 0, j), ("d", 1, j)])
        pos.append(len(queue))
    gu_ready = [pos[(r + n) // _FP - 1] for r, n in blocks]
    d_ready = [pos[(r + n) // _FP - 1 + LAG] for r, n in blocks]
    cum = [0]
    for item in queue:
        cum.append(cum[-1] + item[2])
    waited, started = [0, 0], [LA0, LA1]

    def pump(upto, need=0):
        while waited[1] < min(max(upto, need), len(queue)):
            e = waited[1]
            while waited[0] < (need if e == need - 1 else e - _CFG["HLAG"]):
                queue[waited[0]][1].wait()
                waited[0] += 1
            for cp in queue[e][0]:
                cp.wait()
            waited[1] += 1
            for cls, la in ((1, LA1), (0, LA0)):
                while started[cls] < len(queue) and cum[started[cls]] < cum[e + 1] + 4 * la:
                    assert started[cls] >= wo_phase.n or started[cls] - waited[cls] < _RING
                    for cp in (queue[started[cls]][0] if cls else [queue[started[cls]][1]]):
                        cp.start(priority=cls)
                    started[cls] += 1
        while waited[0] < need:
            queue[waited[0]][1].wait()
            waited[0] += 1

    for i in range(_S // 2):
        pump(3 * i + 2)
        pv(NG - 1, i)

    attn = jnp.zeros((B, D), _F32)
    for t in range(4):
        pump(waited[1] + 4, 16 * (t + 1))
        o = jnp.concatenate([o_ref[4 * i + t] for i in range(8)], axis=-1).astype(_BF16)
        w = wo_buf[:, t * _DH:(t + 1) * _DH, :].reshape(8 * _DH, D)
        attn = attn + jnp.dot(o, w, preferred_element_type=_F32)
    pump(waited[1] + 3)

    x1 = x_buf[...].astype(_F32) + mod(2) * attn
    h2 = (_layernorm(x1) * (1.0 + mod(4)) + mod(3)).astype(_BF16)

    def rows_of(buf, r, n):
        return buf[:, r:r + n, :].reshape(2 * n, D)

    hh = []
    y = jnp.zeros((B, D), _F32)
    n_down = 0

    def down(k):
        return jnp.dot(hh[k], rows_of(wd_buf, *blocks[k]), preferred_element_type=_F32)

    for t, (r, n) in enumerate(blocks):
        pump(waited[1] + 2, gu_ready[t])
        while n_down < len(hh) and d_ready[n_down] <= waited[0]:
            y = y + down(n_down)
            n_down += 1
        gate = lax.dot_general(h2, rows_of(wg_buf, r, n), _NT, preferred_element_type=_F32)
        up = lax.dot_general(h2, rows_of(wu_buf, r, n), _NT, preferred_element_type=_F32)
        hh.append((jax.nn.sigmoid(gate) * up).astype(_BF16))
    for last in _CFG["CUTS"]:
        last += len(blocks)
        pump(0, d_ready[last])
        while n_down <= last:
            y = y + down(n_down)
            n_down += 1
    assert waited == [len(queue)] * 2 and n_down == len(blocks)
    out_ref[...] = (x1 + mod(5) * y).astype(out_ref.dtype)


@jax.jit
def pallas_adaLN_cond__sliding_block_cached__glu_gated_glu__decode_kernel(
    A_x: jax.Array,
    A_k_cache: jax.Array,
    A_v_cache: jax.Array,
    A_wq: jax.Array,
    A_wo: jax.Array,
    B_x: jax.Array,
    B_w_gate: jax.Array,
    B_w_up: jax.Array,
    B_w_down: jax.Array,
    c: jax.Array,
    w_mod: jax.Array,
):
    del B_x
    B, Sq, D = A_x.shape
    Hkv, Sk = A_k_cache.shape[1], A_k_cache.shape[2]
    F = B_w_gate.shape[1]
    assert Sq == 1 and Hkv == _HQ and A_k_cache.shape[3] == _DH
    assert (B, D, Sk) == (8, 512, 4096) and F % (2 * _FP) == 0
    W = min(4096, max(256, Sk // 4))
    NG = B * _HQ // _S

    x = A_x.reshape(B, D)
    k = A_k_cache.reshape(NG, _S, Sk, _DH)
    v = A_v_cache.reshape(NG, _S, Sk, _DH)
    wq = A_wq.reshape(8, D // 8, _HQ * _DH)
    wo = A_wo.reshape(8, _HQ * _DH // 8, D)
    wm = w_mod.reshape(8, D // 8, 6 * D)
    wg = B_w_gate.T.reshape(2, F // 2, D)
    wu = B_w_up.T.reshape(2, F // 2, D)
    wd = B_w_down.reshape(2, F // 2, D)

    any_spec = pl.BlockSpec(memory_space=pl.ANY)
    out = pl.pallas_call(
        functools.partial(_kernel, B=B, D=D, F=F, Sk=Sk, W=W),
        out_shape=jax.ShapeDtypeStruct(x.shape, x.dtype),
        in_specs=[any_spec] * 10,
        out_specs=pl.BlockSpec(memory_space=pltpu.VMEM),
        scratch_shapes=[
            pltpu.VMEM((_S, W, _DH), _BF16),
            pltpu.VMEM((_S, W, _DH), _BF16),
            pltpu.VMEM(wm.shape, _BF16),
            pltpu.VMEM(wq.shape, _BF16),
            pltpu.VMEM(wo.shape, _BF16),
            pltpu.VMEM(wg.shape, _BF16),
            pltpu.VMEM(wu.shape, _BF16),
            pltpu.VMEM(wd.shape, _BF16),
            pltpu.VMEM(x.shape, _BF16),
            pltpu.VMEM(c.shape, _BF16),
            pltpu.VMEM((12, B, 6 * D // 12), _F32),
            pltpu.VMEM((_HQ, B, _DH), _F32),
            pltpu.VMEM((_HQ, B, _DH), _F32),
            pltpu.VMEM((_S, W), _F32),
            pltpu.VMEM((B, D), _F32),
            pltpu.SemaphoreType.DMA((3, _RING)),
            pltpu.SemaphoreType.DMA((2, 3)),
            pltpu.SemaphoreType.DMA((2 + 4 * (F // 2 // _FP + _CFG["LAG"]),)),
        ],
        compiler_params=pltpu.CompilerParams(
            vmem_limit_bytes=64 * 1024 * 1024,
            disable_bounds_checks=not _CFG["CHECKS"],
            disable_semaphore_checks=not _CFG["CHECKS"],
        ),
    )(x, k, v, wq, wo, wg, wu, wd, c, wm)
    return out.reshape(A_x.shape)
```
